```python
import jax
import jax.numpy as jnp

def _softmax(x, axis=-1):
    return jax.nn.softmax(x, axis=axis)
def _gelu(x):
    return jax.nn.gelu(x, approximate=True)
def _silu(x):
    return jax.nn.silu(x)
def _sigmoid(x):
    return jax.nn.sigmoid(x)
def _layernorm(x, axis=-1, eps=1e-5):
    m = jnp.mean(x, axis=axis, keepdims=True)
    v = jnp.var(x, axis=axis, keepdims=True)
    return (x - m) / jnp.sqrt(v + eps)
def _scatter_add(tgt, idx, src, axis=0):
    return tgt.at[idx].add(src)
def _segment_sum(src, seg, n):
    return jax.ops.segment_sum(src, seg, n)
class _Rng:
    def __init__(self, key):
        self._k = key
    def _next(self):
        self._k, sub = jax.random.split(self._k)
        return sub
    def normal(self, shape):
        return jax.random.normal(self._next(), shape, dtype=jnp.bfloat16)
    def randint(self, lo, hi, shape):
        return jax.random.randint(self._next(), shape, lo, hi, dtype=jnp.int32)
    def uniform(self, shape, lo=0.0, hi=1.0):
        return jax.random.uniform(self._next(), shape, jnp.bfloat16, lo, hi)
    def permutation(self, n):
        return jax.random.permutation(self._next(), n)


kernel_name = 'standalone__batchnorm__sampling'

def setup_inputs():
    _rng = _Rng(jax.random.key(int.from_bytes(__import__("os").urandom(4), "little")))
    _w = (lambda a: (lambda t: t.astype(jnp.bfloat16) if jnp.issubdtype(t.dtype, jnp.floating) else t)(jnp.asarray(a)))
    B, S, C = 1024, 32, 576
    K = 3
    return {
        "x": _w((lambda *s: _rng.normal(s) * 0.05)(B, S, C)),
        "w": _w((lambda *s: _rng.normal(s) * 0.05)(K, C, C) * (1.0 / (K * C) ** 0.5)),
        "mean": _w((lambda *s: _rng.normal(s) * 0.05)(C) * 0.1),
        "var": _w(jnp.abs((lambda *s: _rng.normal(s) * 0.05)(C)) + 0.5),
        "g": _w((lambda *s: _rng.normal(s) * 0.05)(C) + 1.0),
        "b": _w((lambda *s: _rng.normal(s) * 0.05)(C) * 0.1),
    }

def reference(x, w, mean, var, g, b):
    K = 3
    P = K // 2
    S = x.shape[1]
    xp = jnp.pad(x, ((0, 0), (P, P), (0, 0)))
    y = sum(jnp.einsum('bsc,cd->bsd', xp[:, k:k + S, :], w[k]) for k in range(K))
    inv_std = 1.0 / jnp.sqrt(var + 1e-5)
    y = (y - mean) * (g * inv_std) + b
    return _silu(y)
```

```python
import functools
import jax
import jax.numpy as jnp
import jax.experimental.pallas as pl
import jax.experimental.pallas.tpu as pltpu

A_ = 2.0 / 3.0
B_ = 1.5
A2 = A_ * A_
B2 = B_ * B_
NA = 2 * A2 * (A2 - B2)
NB = 2 * B2 * (B2 - A2)


def build(TB=128):
    def fn(x, w, mean, var, g, b):
        Bn, S, C = x.shape
        xt = jnp.transpose(x, (1, 2, 0))
        wt = jnp.transpose(w, (0, 2, 1))
        col = lambda v: v.reshape(C, 1)
        NT = S // 4

        def kernel(x_ref, w_ref, mean_ref, var_ref, g_ref, b_ref, o_ref, gt_ref, sc_ref, sh_ref):
            @pl.when(pl.program_id(0) == 0)
            def _():
                w0 = w_ref[0].astype(jnp.float32)
                w1 = w_ref[1].astype(jnp.float32)
                w2 = w_ref[2].astype(jnp.float32)
                gt_ref[0] = w_ref[0]
                gt_ref[5] = w_ref[2]
                ea = (w0 + A2 * w2) * (1.0 / NA)
                oa = w1 * (A_ / NA)
                gt_ref[1] = (ea + oa).astype(jnp.bfloat16)
                gt_ref[2] = (ea - oa).astype(jnp.bfloat16)
                eb = (w0 + B2 * w2) * (1.0 / NB)
                ob = w1 * (B_ / NB)
                gt_ref[3] = (eb + ob).astype(jnp.bfloat16)
                gt_ref[4] = (eb - ob).astype(jnp.bfloat16)
                sc = 0.5 * g_ref[...].astype(jnp.float32) * jax.lax.rsqrt(var_ref[...].astype(jnp.float32) + 1e-5)
                sh = 0.5 * b_ref[...].astype(jnp.float32) - mean_ref[...].astype(jnp.float32) * sc
                sc_ref[...] = jnp.broadcast_to(sc, sc_ref.shape)
                sh_ref[...] = jnp.broadcast_to(sh, sh_ref.shape)

            def body(t, carry):
                f32 = jnp.float32
                s0 = t * 4
                lo = jnp.maximum(s0 - 1, 0)
                hi = jnp.minimum(s0 + 4, S - 1)
                d0 = jnp.where(t > 0, x_ref[lo].astype(f32), 0.0)
                d1 = x_ref[s0].astype(f32)
                d2 = x_ref[s0 + 1].astype(f32)
                d3 = x_ref[s0 + 2].astype(f32)
                d4 = x_ref[s0 + 3].astype(f32)
                d5 = jnp.where(t < NT - 1, x_ref[hi].astype(f32), 0.0)
                u = A2 * d2
                v = B2 * d2
                P = d4 - v
                Pp = d4 - u
                t0 = (d0 - u) + P
                up = A2 * d3
                vp = B2 * d3
                R = d1 - up
                Rp = d1 - vp
                t5 = (d5 - vp) + R
                bR = B_ * R
                aRp = A_ * Rp
                t1 = P - bR
                t2 = P + bR
                t3 = Pp - aRp
                t4 = Pp + aRp
                bf = jnp.bfloat16
                m = [jnp.dot(gt_ref[i], tt.astype(bf), preferred_element_type=f32)
                     for i, tt in enumerate((t0, t1, t2, t3, t4, t5))]
                s12 = m[1] + m[2]
                d12 = m[1] - m[2]
                s34 = m[3] + m[4]
                d34 = m[3] - m[4]
                y0 = m[0] + s12 + s34
                p = A_ * d12
                q = B_ * d34
                y1 = p + q
                y2 = A2 * s12 + B2 * s34
                y3 = A2 * p + B2 * q + m[5]
                sc = sc_ref[...]
                sh = sh_ref[...]
                for j, y in enumerate((y0, y1, y2, y3)):
                    h = y * sc + sh
                    o_ref[s0 + j] = (h + h * jnp.tanh(h)).astype(o_ref.dtype)
                return carry

            jax.lax.fori_loop(0, NT, body, 0)

        vec = pl.BlockSpec((C, 1), lambda i: (0, 0))
        out = pl.pallas_call(
            kernel,
            grid=(Bn // TB,),
            in_specs=[
                pl.BlockSpec((S, C, TB), lambda i: (0, 0, i)),
                pl.BlockSpec((3, C, C), lambda i: (0, 0, 0)),
                vec, vec, vec, vec,
            ],
            out_specs=pl.BlockSpec((S, C, TB), lambda i: (0, 0, i)),
            out_shape=jax.ShapeDtypeStruct((S, C, Bn), x.dtype),
            scratch_shapes=[
                pltpu.VMEM((6, C, C), jnp.bfloat16),
                pltpu.VMEM((C, TB), jnp.float32),
                pltpu.VMEM((C, TB), jnp.float32),
            ],
            compiler_params=pltpu.CompilerParams(
                dimension_semantics=("arbitrary",),
                vmem_limit_bytes=100 * 1024 * 1024,
            ),
        )(xt, wt, col(mean), col(var), col(g), col(b))
        return jnp.transpose(out, (2, 0, 1))
    return fn


@jax.jit
def pallas_standalone__batchnorm__sampling_kernel(x, w, mean, var, g, b):
    return build()(x, w, mean, var, g, b)
```

```python
import functools
import jax
import jax.numpy as jnp
from jax import lax
import jax.experimental.pallas as pl
import jax.experimental.pallas.tpu as pltpu

A_ = 2.0 / 3.0
B_ = 1.5
A2 = A_ * A_
B2 = B_ * B_
NA = 2 * A2 * (A2 - B2)
NB = 2 * B2 * (B2 - A2)
L = 128
f32 = jnp.float32
bf16 = jnp.bfloat16
u32 = jnp.uint32


def _divmod_pow2(x, n):
    if isinstance(x, int):
        return x // n, x % n
    sh = n.bit_length() - 1
    assert 1 << sh == n
    return lax.shift_right_logical(x, sh), lax.bitwise_and(x, n - 1)


def build(NT=2, nodma=False, nit=None, nobc=True, vec1d=True, midout=True, mode='jit', order=(1,2,3,4,0,5), carry=True, xs1=1):
    def fn(x, w, mean, var, g, b):
        Bn, S, C = x.shape
        xt = jnp.transpose(x, (1, 2, 0))
        NJ = Bn // L
        TPS = S // 4
        NCH = NJ * TPS
        NIT = NCH // NT
        KF = (C // L) * L
        KR = C - KF
        NK = KF // L
        NX = 2 * NT + 1
        NSEM = 8 if NX <= 8 else 16
        assert NX <= NSEM

        def kernel(x_hbm, w_hbm, mean_hbm, var_hbm, g_hbm, b_hbm, o_hbm,
                   xbuf, obuf, wbuf, vb0, vb1, vb2, vb3, gcols, abuf, sc_ref, sh_ref, dummy, in_sems, w_sems, v_sems, out_sem):
            def in_copy(c):
                j, t = _divmod_pow2(c, TPS)
                js = _divmod_pow2(j, NJ)[1]
                return pltpu.make_async_copy(
                    x_hbm.at[pl.ds(t * 4, 4), :, pl.ds(pl.multiple_of(js * L, L), L)],
                    xbuf.at[j, pl.ds(t * 4 + 1, 4)],
                    in_sems.at[_divmod_pow2(c, NSEM)[1]])

            def out_copy(n):
                j, t = _divmod_pow2(n, TPS)
                return pltpu.make_async_copy(
                    obuf.at[j, pl.ds(t * 4, 4)],
                    o_hbm.at[pl.ds(t * 4, 4), :, pl.ds(pl.multiple_of(j * L, L), L)],
                    out_sem)

            kchunks = [(kc * L, L) for kc in range(NK)] + [(KF, KR)]
            w_copies = [pltpu.make_async_copy(w_hbm.at[:, pl.ds(c0, n), :], wbuf.at[:, pl.ds(c0, n), :], w_sems.at[i])
                        for i, (c0, n) in enumerate(kchunks)]
            vbuf = (vb0, vb1, vb2, vb3)
            v_copies = [pltpu.make_async_copy(r, vbuf[i], v_sems.at[i])
                        for i, r in enumerate((mean_hbm, var_hbm, g_hbm, b_hbm))]
            for cp in w_copies:
                cp.start()
            for cp in v_copies:
                cp.start()

            z = jnp.zeros((C // 2, L), u32)
            xu = xbuf.bitcast(u32)
            for j in range(NJ + 1):
                xu[j, 0] = z
                if j < NJ:
                    xu[j, S + 1] = z

            def tr(k, c0, n):
                return wbuf[k, c0:c0 + n, :].astype(f32).T

            def gs(w0, w1, w2):
                ea = (w0 + A2 * w2) * (1.0 / NA)
                oa = w1 * (A_ / NA)
                eb = (w0 + B2 * w2) * (1.0 / NB)
                ob = w1 * (B_ / NB)
                return [w0, ea + oa, ea - oa, eb + ob, eb - ob, w2]

            for kc in range(NK):
                w_copies[kc].wait()
                if not nodma:
                    if kc == xs1:
                        for c in range(NT + 1):
                            in_copy(c).start()
                    if kc == 3:
                        for c in range(NT + 1, NX):
                            in_copy(c).start()
                w0, w1, w2 = (tr(k, kc * L, L) for k in range(3))
                for i, gi in enumerate(gs(w0, w1, w2)):
                    gcols[5 * i + kc] = gi.astype(bf16)
            w_copies[NK].wait()
            w0, w1, w2 = (tr(k, KF, KR) for k in range(3))
            gr = gs(w0, w1, w2)
            ca = w0 * (-1.0 / NA)
            cb = w0 * (-1.0 / NB)
            for i, extra in ((1, ca), (2, ca), (3, cb), (4, cb), (5, jnp.zeros_like(w0))):
                gcols[5 * i + NK] = jnp.concatenate([gr[i], extra], axis=1).astype(bf16)

            for cp in v_copies:
                cp.wait()
            ld = lambda i: vbuf[i][...].astype(f32).reshape(1, C)
            mean_v, var_v, g_v, b_v = (ld(i) for i in range(4))
            sc = 0.5 * g_v * lax.rsqrt(var_v + 1e-5)
            sh = 0.5 * b_v - mean_v * sc
            sc_ref[...] = jnp.broadcast_to(sc, (L, C)).T
            sh_ref[...] = jnp.broadcast_to(sh, (L, C)).T

            gu = gcols.bitcast(u32)
            au = abuf.bitcast(u32)

            def transform(n):
                j, t = _divmod_pow2(n, TPS)
                s0 = t * 4
                d0, d1, d2, d3, d4, d5 = (xbuf[j, s0 + q].astype(f32) for q in range(6))
                uu = A2 * d2
                v = B2 * d2
                P = d4 - v
                Pp = d4 - uu
                t0 = (d0 - uu) + P
                up = A2 * d3
                vp = B2 * d3
                R = d1 - up
                Rp = d1 - vp
                t5 = (d5 - vp) + R
                bR = B_ * R
                aRp = A_ * Rp
                return (t0, P - bR, P + bR, Pp - aRp, Pp + aRp, t5)

            S2 = A2 + B2

            def t_jit(n, i, lo=0, hi=None):
                hi = C if hi is None else hi
                j, t = _divmod_pow2(n, TPS)
                s0 = t * 4
                d = lambda q: xbuf[j, s0 + q, lo:hi, :].astype(f32)
                if i == 0:
                    return (d(0) + d(4)) - S2 * d(2)
                if i == 5:
                    return (d(1) + d(5)) - S2 * d(3)
                c2, c1, c3 = {1: (B2, -B_, A_), 2: (B2, B_, -A_), 3: (A2, -A_, B_), 4: (A2, A_, -B_)}[i]
                return (d(4) - c2 * d(2)) + (c1 * d(1) + c3 * d(3))

            def lhs_for(i):
                nk = NK if i == 0 else NK + 1
                return jnp.concatenate([pltpu.bitcast(gu[5 * i + kc], bf16) for kc in range(nk)], axis=1)

            def matmuls_jit(n, first_from_abuf):
                m = [None] * 6
                for idx, i in enumerate(order):
                    if idx == 0 and first_from_abuf:
                        rhs = pltpu.bitcast(au[0, :(KF if i == 0 else KF + L) // 2, :], bf16)
                    else:
                        rhs = rhs_jit(n, i)
                    m[i] = jnp.dot(lhs_for(i), rhs, preferred_element_type=f32)
                    if mode == 'jit':
                        dummy[0] = idx
                return m

            def rhs_jit(n, i):
                if i == 0:
                    return t_jit(n, 0, 0, KF).astype(bf16)
                return jnp.concatenate([t_jit(n, i), t_jit(n, 0, KF, C)], axis=0).astype(bf16)

            def store_first(n):
                i = order[0]
                abuf[0, :(KF if i == 0 else KF + L), :] = rhs_jit(n, i)

            def epilogue(n, m):
                j, t = _divmod_pow2(n, TPS)
                s0 = t * 4
                sc = sc_ref[...]
                sh = sh_ref[...]
                s12 = m[1] + m[2]
                d12 = m[1] - m[2]
                s34 = m[3] + m[4]
                d34 = m[3] - m[4]
                y0 = m[0] + s12 + s34
                p = A_ * d12
                q = B_ * d34
                y1 = p + q
                y2 = A2 * s12 + B2 * s34
                y3 = A2 * p + B2 * q + m[5]
                for jj, y in enumerate((y0, y1, y2, y3)):
                    h = y * sc + sh
                    obuf[j, s0 + jj] = (h + h * jnp.tanh(h)).astype(bf16)

            if not nodma:
                in_copy(0).wait()
            if carry:
                assert order[0] != 5
                store_first(0)
            if not nodma:
                for c in range(1, NT + 1):
                    in_copy(c).wait()

            def body(it, cc):
                c0 = it * NT
                for u in range(NT):
                    m = matmuls_jit(c0 + u, carry and u == 0)
                    if u == NT - 1 and carry:
                        store_first(c0 + NT)
                    epilogue(c0 + u, m)
                    if midout and not nodma:
                        out_copy(c0 + u).start()
                if not nodma:
                    for u in range(NT):
                        in_copy(c0 + NX + u).start()
                    for u in range(NT):
                        in_copy(c0 + NT + 1 + u).wait()
                if not nodma and not midout:
                    for u in range(NT):
                        out_copy(c0 + u).start()
                return cc

            lax.fori_loop(0, NIT if nit is None else nit, body, 0)
            if not nodma:
                for c in range(NCH + NT + 1, NCH + NX):
                    in_copy(c).wait()
                pltpu.make_async_copy(obuf, obuf, out_sem).wait()

        anyspec = pl.BlockSpec(memory_space=pl.ANY)
        row = (lambda v: v) if vec1d else (lambda v: v.reshape(1, C))
        out = pl.pallas_call(
            kernel,
            in_specs=[anyspec] * 6,
            out_specs=anyspec,
            out_shape=jax.ShapeDtypeStruct((S, C, Bn), x.dtype),
            scratch_shapes=[
                pltpu.VMEM((NJ + 2, S + 2, C, L), bf16),
                pltpu.VMEM((NJ, S, C, L), bf16),
                pltpu.VMEM((3, C, C), bf16),
                *[pltpu.VMEM((C,) if vec1d else (1, C), bf16)] * 4,
                pltpu.VMEM((30, C, L), bf16),
                pltpu.VMEM((1, KF + L, L), bf16),
                pltpu.VMEM((C, L), f32),
                pltpu.VMEM((C, L), f32),
                pltpu.SMEM((1,), jnp.int32),
                pltpu.SemaphoreType.DMA((NSEM,)),
                pltpu.SemaphoreType.DMA((NK + 1,)),
                pltpu.SemaphoreType.DMA((4,)),
                pltpu.SemaphoreType.DMA(()),
            ],
            compiler_params=pltpu.CompilerParams(
                vmem_limit_bytes=110 * 1024 * 1024,
                disable_bounds_checks=nobc,
            ),
        )(xt, w, row(mean), row(var), row(g), row(b))
        return jnp.transpose(out, (2, 0, 1))
    return fn


@jax.jit
def pallas_standalone__batchnorm__sampling_kernel(x, w, mean, var, g, b):
    return build()(x, w, mean, var, g, b)
```

```python
import jax
import jax.numpy as jnp
from jax import lax
import jax.experimental.pallas as pl
import jax.experimental.pallas.tpu as pltpu

A_ = 2.0 / 3.0
B_ = 1.5
A2 = A_ * A_
B2 = B_ * B_
S2 = A2 + B2
NA = 2 * A2 * (A2 - B2)
NB = 2 * B2 * (B2 - A2)
L = 128
f32 = jnp.float32
bf16 = jnp.bfloat16
u32 = jnp.uint32


def _divmod_pow2(x, n):
    if isinstance(x, int):
        return x // n, x % n
    sh = n.bit_length() - 1
    assert 1 << sh == n
    return lax.shift_right_logical(x, sh), lax.bitwise_and(x, n - 1)


def build(P=4, NT=4, order=(1, 2, 3, 4, 0, 5), nA=2, nC=3, nit=None, spu=0, noout=False, pair=False,
          carry0=False, lastsplit=None, pin=False, merge=True, stg=(1, 0)):
    def fn(x, w, mean, var, g, b):
        Bn, S, C = x.shape
        xt = jnp.transpose(x, (1, 2, 0))
        NJ = Bn // L
        TPS = S // 4
        NU = NJ * TPS
        KF = (C // L) * L
        KR = C - KF
        NK = KF // L
        PP = 4 * (P + 1) if carry0 else 4 * P + 1
        assert (NU - P) % NT == 0
        NIT = (NU - P) // NT
        NSEM = 16
        assert NT + 1 <= NSEM // 2

        def kernel(x_hbm, w_hbm, mean_hbm, var_hbm, g_hbm, b_hbm, o_hbm,
                   xbuf, obuf, wbuf, vb0, vb1, vb2, vb3, gcols, abuf, acc, sc_ref, sh_ref, dummy,
                   x_sems, p_sems, w_sems, v_sems, out_sem):
            def lanes(j):
                return pl.ds(j * L if isinstance(j, int) else pl.multiple_of(j * L, L), L)

            def x_copy(j, p0, n, sem, r0=0, r1=C):
                return pltpu.make_async_copy(
                    x_hbm.at[pl.ds(p0, n), pl.ds(r0, r1 - r0), lanes(j)],
                    xbuf.at[j, pl.ds(p0 + 1, n), pl.ds(r0, r1 - r0), :], sem)

            def chunk(c, cnt=1, sem=None):
                j, t = _divmod_pow2(c, TPS)
                j = _divmod_pow2(j, NJ)[1]
                sem = _divmod_pow2(c, NSEM)[1] if sem is None else sem
                return x_copy(j, 4 * t, 4 * cnt, x_sems.at[sem])

            def window(c):
                if merge:
                    assert NT == 4 and P == 4
                    return [chunk(c, 3, 0), chunk(c + 3, 1, 1)]
                return [chunk(c + u) for u in range(NT)]

            def out_copy(n, p0=0, cnt=4):
                j, t = _divmod_pow2(n, TPS)
                return pltpu.make_async_copy(
                    obuf.at[j, pl.ds(t * 4 + p0, cnt)], o_hbm.at[pl.ds(t * 4 + p0, cnt), :, lanes(j)], out_sem)

            kchunks = [(kc * L, L) for kc in range(NK)] + [(KF, KR)]
            wc = [pltpu.make_async_copy(w_hbm.at[:, pl.ds(c0, n), :], wbuf.at[:, pl.ds(c0, n), :], w_sems.at[i])
                  for i, (c0, n) in enumerate(kchunks)]
            vbuf = (vb0, vb1, vb2, vb3)
            vc = [pltpu.make_async_copy(r, vbuf[i], v_sems.at[i])
                  for i, r in enumerate((mean_hbm, var_hbm, g_hbm, b_hbm))]
            xa = [x_copy(0, 0, PP, p_sems.at[0], 0, L), x_copy(0, 0, PP, p_sems.at[1], L, 2 * L),
                  x_copy(0, 0, PP, p_sems.at[2], 2 * L, C)]
            pre = [] if carry0 else [x_copy(0, PP, 3, p_sems.at[3])]
            pre += window(P + 1)

            for cp in [wc[0], xa[0], wc[1], *vc, xa[1], wc[2], wc[3], wc[4], xa[2], *pre]:
                cp.start()

            z = jnp.zeros((C // 2, L), u32)
            xu = xbuf.bitcast(u32)
            for j in range(NJ):
                xu[j, 0] = z
                xu[j, S + 1] = z

            def setup(kc):
                if kc < NK:
                    blk = [wbuf[k, kc * L:(kc + 1) * L, :].astype(f32) for k in range(3)]
                else:
                    r = [wbuf[k, KF:, :].astype(f32) for k in range(3)]
                    zz = jnp.zeros_like(r[0])
                    blk = [jnp.concatenate([r[0], -r[0]], axis=0), jnp.concatenate([r[1], zz], axis=0),
                           jnp.concatenate([r[2], zz], axis=0)]
                w0, w1, w2 = (t.T for t in blk)
                ea = (w0 + A2 * w2) * (1.0 / NA)
                oa = w1 * (A_ / NA)
                eb = (w0 + B2 * w2) * (1.0 / NB)
                ob = w1 * (B_ / NB)
                for i, gi in enumerate([w0, ea + oa, ea - oa, eb + ob, eb - ob, w2]):
                    if i > 0 or kc < NK:
                        gcols[5 * i + kc] = gi.astype(bf16)

            def bn_consts():
                ld = lambda i: vbuf[i][...].astype(f32).reshape(1, C)
                mean_v, var_v, g_v, b_v = (ld(i) for i in range(4))
                sc = 0.5 * g_v * lax.rsqrt(var_v + 1e-5)
                sh = 0.5 * b_v - mean_v * sc
                sc_ref[...] = jnp.broadcast_to(sc, (L, C)).T
                sh_ref[...] = jnp.broadcast_to(sh, (L, C)).T

            gu = gcols.bitcast(u32)
            au = abuf.bitcast(u32)

            def dload(n, lo, hi):
                j, t = _divmod_pow2(n, TPS)
                j = _divmod_pow2(j, NJ)[1]
                return lambda q: xbuf[j, 4 * t + q, lo:hi, :].astype(f32)

            def t_jit(n, i, lo, hi):
                d = dload(n, lo, hi)
                if i == 0:
                    return (d(0) + d(4)) - S2 * d(2)
                if i == 5:
                    return (d(1) + d(5)) - S2 * d(3)
                c2, c1, c3 = {1: (B2, -B_, A_), 2: (B2, B_, -A_), 3: (A2, -A_, B_), 4: (A2, A_, -B_)}[i]
                return (d(4) - c2 * d(2)) + (c1 * d(1) + c3 * d(3))

            def lhs_for(i, k0=0):
                nk = NK if i == 0 else NK + 1
                return jnp.concatenate([pltpu.bitcast(gu[5 * i + kc], bf16) for kc in range(k0, nk)], axis=1)

            def rhs_jit(n, i, k0=0):
                if i == 0:
                    return t_jit(n, 0, k0 * L, KF).astype(bf16)
                return jnp.concatenate([t_jit(n, i, k0 * L, C), t_jit(n, 0, KF, C)], axis=0).astype(bf16)

            def rhs_pair(n, i, k0=0):
                d = dload(n, k0 * L, C)
                c2, c1, c3 = {1: (B2, -B_, A_), 3: (A2, -A_, B_)}[i]
                e = d(4) - c2 * d(2)
                o = c1 * d(1) + c3 * d(3)
                t0r = t_jit(n, 0, KF, C)
                return [jnp.concatenate([v, t0r], axis=0).astype(bf16) for v in (e + o, e - o)]

            def fence(v):
                dummy[0] = v

            def matmuls(n, first_from_abuf, k0=0, stage=None):
                m = [None] * 6
                held = {}
                for idx, i in enumerate(order):
                    if idx == 0 and first_from_abuf:
                        rhs = pltpu.bitcast(au[...], bf16)
                    elif idx == stage:
                        abuf[...] = rhs_jit(n, i, k0)
                        rhs = pltpu.bitcast(au[...], bf16)
                    elif i in held:
                        rhs = held[i]
                    elif pair and i in (1, 3):
                        rhs, held[i + 1] = rhs_pair(n, i, k0)
                    else:
                        rhs = rhs_jit(n, i, k0)
                    m[i] = jnp.dot(lhs_for(i, k0), rhs, preferred_element_type=f32)
                    if k0:
                        m[i] = m[i] + acc[i, :, n * L:(n + 1) * L]
                    fence(idx)
                return m

            def epilogue(n, m, split=None):
                j, t = _divmod_pow2(n, TPS)
                sc = sc_ref[...]
                sh = sh_ref[...]
                s12 = m[1] + m[2]
                d12 = m[1] - m[2]
                s34 = m[3] + m[4]
                d34 = m[3] - m[4]
                y0 = m[0] + s12 + s34
                p = A_ * d12
                q = B_ * d34
                y1 = p + q
                y2 = A2 * s12 + B2 * s34
                y3 = A2 * p + B2 * q + m[5]
                ys = (y0, y1, y2, y3)
                for p0, cnt in (split or ((0, 4),)):
                    for jj in range(p0, p0 + cnt):
                        h = ys[jj] * sc + sh
                        obuf[j, 4 * t + jj] = (h + h * jnp.tanh(h)).astype(bf16)
                    if not noout:
                        out_copy(n, p0, cnt).start()

            def kmajor(kc, comps):
                for i in comps:
                    rhs = jnp.concatenate(
                        [t_jit(n, i, kc * L, (kc + 1) * L) for n in range(P)], axis=1).astype(bf16)
                    r = jnp.dot(pltpu.bitcast(gu[5 * i + kc], bf16), rhs, preferred_element_type=f32)
                    acc[i] = r if kc == 0 else acc[i] + r
                    fence(i)

            comps = (0, 5, 1, 2, 3, 4)
            wc[0].wait()
            setup(0)
            xa[0].wait()
            kmajor(0, comps[:nA])
            wc[1].wait()
            kmajor(0, comps[nA:])
            setup(1)
            xa[1].wait()
            wc[2].wait()
            for cp in vc:
                cp.wait()
            kmajor(1, comps[:nC])
            setup(2)
            bn_consts()
            wc[3].wait()
            wc[4].wait()
            kmajor(1, comps[nC:])
            setup(3)
            setup(4)
            xa[2].wait()
            for n in range(P):
                m = matmuls(n, False, k0=2)
                if n == P - 1 and carry0:
                    abuf[...] = rhs_jit(P, order[0])
                epilogue(n, m)
            for cp in pre:
                cp.wait()
            if not carry0:
                abuf[...] = rhs_jit(P, order[0])

            def body(it, cc):
                c0 = P + it * NT
                nxt = window(c0 + NT + 1)
                if spu == 0:
                    for cp in nxt:
                        cp.start()
                for u in range(NT):
                    m = matmuls(c0 + u, u == 0, stage=stg[1] if (stg and u == NT - stg[0]) else None)
                    for cp in nxt[u * spu:(u + 1) * spu]:
                        cp.start()
                    if u == NT - 1:
                        if pin:
                            xu[0, 0, 0:8, :] = jnp.zeros((8, L), u32)
                        abuf[...] = rhs_jit(c0 + NT, order[0])
                    epilogue(c0 + u, m, lastsplit if u == NT - 1 else None)
                for cp in nxt:
                    cp.wait()
                return cc

            lax.fori_loop(0, NIT if nit is None else nit, body, 0)
            if not noout:
                if nit is None:
                    pltpu.make_async_copy(obuf, obuf, out_sem).wait()
                else:
                    for n in range(P + nit * NT):
                        out_copy(0).wait()

        anyspec = pl.BlockSpec(memory_space=pl.ANY)
        out = pl.pallas_call(
            kernel,
            in_specs=[anyspec] * 6,
            out_specs=anyspec,
            out_shape=jax.ShapeDtypeStruct((S, C, Bn), x.dtype),
            scratch_shapes=[
                pltpu.VMEM((NJ, S + 2, C, L), bf16),
                pltpu.VMEM((NJ, S, C, L), bf16),
                pltpu.VMEM((3, C, C), bf16),
                *[pltpu.VMEM((C,), bf16)] * 4,
                pltpu.VMEM((30, C, L), bf16),
                pltpu.VMEM((KF + L, L), bf16),
                pltpu.VMEM((6, C, P * L), f32),
                pltpu.VMEM((C, L), f32),
                pltpu.VMEM((C, L), f32),
                pltpu.SMEM((1,), jnp.int32),
                pltpu.SemaphoreType.DMA((NSEM,)),
                pltpu.SemaphoreType.DMA((4,)),
                pltpu.SemaphoreType.DMA((NK + 1,)),
                pltpu.SemaphoreType.DMA((4,)),
                pltpu.SemaphoreType.DMA(()),
            ],
            compiler_params=pltpu.CompilerParams(
                vmem_limit_bytes=120 * 1024 * 1024,
                disable_bounds_checks=True,
            ),
        )(xt, w, mean, var, g, b)
        return jnp.transpose(out, (2, 0, 1))
    return fn


@jax.jit
def pallas_standalone__batchnorm__sampling_kernel(x, w, mean, var, g, b):
    return build()(x, w, mean, var, g, b)
```

```python
import jax
import jax.numpy as jnp
from jax import lax
import jax.experimental.pallas as pl
import jax.experimental.pallas.tpu as pltpu

A_ = 2.0 / 3.0
B_ = 1.5
A2 = A_ * A_
B2 = B_ * B_
S2 = A2 + B2
NA = 2 * A2 * (A2 - B2)
NB = 2 * B2 * (B2 - A2)
L = 128
f32 = jnp.float32
bf16 = jnp.bfloat16
u32 = jnp.uint32


def _divmod_pow2(x, n):
    if isinstance(x, int):
        return x // n, x % n
    sh = n.bit_length() - 1
    assert 1 << sh == n
    return lax.shift_right_logical(x, sh), lax.bitwise_and(x, n - 1)


def build(P=4, NT=6, order=(1, 2, 3, 4, 5, 0), nA=2, nC=3, nit=None, spu=0, noout=False, pair=False,
          carry0=False, lastsplit=((1, 2), (3, 1), (0, 1)), pin=False, merge=True, stg=(1, 0), scopes=False, KM=2, nosc=True, defer=True,
          fifo='w0 v x0 w1 x1 w2 w3 w4 x2',
          plan=(('w0 v', 's0 bn'), ('x0', 'm05'), ('w1 x1 w2', 's1 s2 m01 m13'), ('w3 w4', 's3 s4 m13'), ('x2 xh', ''))):
    import contextlib
    scope = jax.named_scope if scopes else (lambda n: contextlib.nullcontext())

    def fn(x, w, mean, var, g, b):
        Bn, S, C = x.shape
        xt = jnp.transpose(x, (1, 2, 0))
        NJ = Bn // L
        TPS = S // 4
        NU = NJ * TPS
        KF = (C // L) * L
        KR = C - KF
        NK = KF // L
        PP = 4 * (P + 1) if carry0 else 4 * P + 1
        assert (NU - P) % NT == 0
        NIT = (NU - P) // NT
        NSEM = (2 if NT == 4 else NT // 2 + 1) if merge else 16

        def kernel(x_hbm, w_hbm, mean_hbm, var_hbm, g_hbm, b_hbm, o_hbm,
                   xbuf, obuf, wbuf, vb0, vb1, vb2, vb3, gcols, abuf, acc, sc_ref, sh_ref, dummy,
                   x_sems, p_sems, w_sems, v_sems, out_sem):
            def lanes(j):
                return pl.ds(j * L if isinstance(j, int) else pl.multiple_of(j * L, L), L)

            def x_copy(j, p0, n, sem, r0=0, r1=C):
                return pltpu.make_async_copy(
                    x_hbm.at[pl.ds(p0, n), pl.ds(r0, r1 - r0), lanes(j)],
                    xbuf.at[j, pl.ds(p0 + 1, n), pl.ds(r0, r1 - r0), :], sem)

            def chunk(c, cnt=1, sem=None):
                j, t = _divmod_pow2(c, TPS)
                j = _divmod_pow2(j, NJ)[1]
                sem = _divmod_pow2(c, NSEM)[1] if sem is None else sem
                return x_copy(j, 4 * t, 4 * cnt, x_sems.at[sem])

            def window(c):
                if merge and NT == 4:
                    assert P == 4
                    return [chunk(c, 3, 0), chunk(c + 3, 1, 1)]
                if merge:
                    assert NT % 2 == 0 and P % 2 == 0
                    return ([chunk(c, 1, 0)] + [chunk(c + u, 2, 1 + u // 2) for u in range(1, NT - 1, 2)]
                            + [chunk(c + NT - 1, 1, NT // 2)])
                return [chunk(c + u) for u in range(NT)]

            def out_copy(n, p0=0, cnt=4):
                j, t = _divmod_pow2(n, TPS)
                return pltpu.make_async_copy(
                    obuf.at[j, pl.ds(t * 4 + p0, cnt)], o_hbm.at[pl.ds(t * 4 + p0, cnt), :, lanes(j)], out_sem)

            kchunks = [(kc * L, L) for kc in range(NK)] + [(KF, KR)]
            wc = [pltpu.make_async_copy(w_hbm.at[:, pl.ds(c0, n), :], wbuf.at[:, pl.ds(c0, n), :], w_sems.at[i])
                  for i, (c0, n) in enumerate(kchunks)]
            vbuf = (vb0, vb1, vb2, vb3)
            vc = [pltpu.make_async_copy(r, vbuf[i], v_sems.at[i])
                  for i, r in enumerate((mean_hbm, var_hbm, g_hbm, b_hbm))]
            xa = [x_copy(0, 0, PP, p_sems.at[kc], kc * L, (kc + 1) * L if kc < KM else C) for kc in range(KM + 1)]
            pre = [x_copy(0, PP, 3, p_sems.at[KM + 1])]
            pre += window(P + 1)

            nm0 = dict(w0=[wc[0]], w1=[wc[1]], w2=[wc[2]], w3=[wc[3]], w4=[wc[4]], v=vc,
                       **{f'x{i}': [cp] for i, cp in enumerate(xa)})
            for nm in fifo.split():
                for cp in nm0[nm]:
                    cp.start()
            for cp in pre:
                cp.start()

            z = jnp.zeros((C // 2, L), u32)
            xu = xbuf.bitcast(u32)
            for j in range(NJ):
                xu[j, 0] = z
                xu[j, S + 1] = z

            def setup(kc):
                if kc < NK:
                    blk = [wbuf[k, kc * L:(kc + 1) * L, :].astype(f32) for k in range(3)]
                else:
                    r = [wbuf[k, KF:, :].astype(f32) for k in range(3)]
                    zz = jnp.zeros_like(r[0])
                    blk = [jnp.concatenate([r[0], -r[0]], axis=0), jnp.concatenate([r[1], zz], axis=0),
                           jnp.concatenate([r[2], zz], axis=0)]
                w0, w1, w2 = (t.T for t in blk)
                ea = (w0 + A2 * w2) * (1.0 / NA)
                oa = w1 * (A_ / NA)
                eb = (w0 + B2 * w2) * (1.0 / NB)
                ob = w1 * (B_ / NB)
                for i, gi in enumerate([w0, ea + oa, ea - oa, eb + ob, eb - ob, w2]):
                    if i > 0 or kc < NK:
                        gcols[5 * i + kc] = gi.astype(bf16)

            def bn_consts():
                ld = lambda i: vbuf[i][...].astype(f32).reshape(1, C)
                mean_v, var_v, g_v, b_v = (ld(i) for i in range(4))
                sc = 0.5 * g_v * lax.rsqrt(var_v + 1e-5)
                sh = 0.5 * b_v - mean_v * sc
                sc_ref[...] = jnp.broadcast_to(sc, (L, C)).T
                sh_ref[...] = jnp.broadcast_to(sh, (L, C)).T

            gu = gcols.bitcast(u32)
            au = abuf.bitcast(u32)

            def dload(n, lo, hi):
                j, t = _divmod_pow2(n, TPS)
                j = _divmod_pow2(j, NJ)[1]
                return lambda q: xbuf[j, 4 * t + q, lo:hi, :].astype(f32)

            def t_jit(n, i, lo, hi):
                d = dload(n, lo, hi)
                if i == 0:
                    return (d(0) + d(4)) - S2 * d(2)
                if i == 5:
                    return (d(1) + d(5)) - S2 * d(3)
                c2, c1, c3 = {1: (B2, -B_, A_), 2: (B2, B_, -A_), 3: (A2, -A_, B_), 4: (A2, A_, -B_)}[i]
                return (d(4) - c2 * d(2)) + (c1 * d(1) + c3 * d(3))

            def lhs_for(i, k0=0):
                nk = NK if i == 0 else NK + 1
                return jnp.concatenate([pltpu.bitcast(gu[5 * i + kc], bf16) for kc in range(k0, nk)], axis=1)

            def rhs_jit(n, i, k0=0):
                if i == 0:
                    return t_jit(n, 0, k0 * L, KF).astype(bf16)
                return jnp.concatenate([t_jit(n, i, k0 * L, C), t_jit(n, 0, KF, C)], axis=0).astype(bf16)

            def rhs_pair(n, i, k0=0):
                d = dload(n, k0 * L, C)
                c2, c1, c3 = {1: (B2, -B_, A_), 3: (A2, -A_, B_)}[i]
                e = d(4) - c2 * d(2)
                o = c1 * d(1) + c3 * d(3)
                t0r = t_jit(n, 0, KF, C)
                return [jnp.concatenate([v, t0r], axis=0).astype(bf16) for v in (e + o, e - o)]

            def fence(v):
                dummy[0] = v

            def matmuls(n, first_from_abuf, k0=0, stage=None):
                m = [None] * 6
                held = {}
                for idx, i in enumerate(order):
                    if idx == 0 and first_from_abuf:
                        rhs = pltpu.bitcast(au[...], bf16)
                    elif idx == stage:
                        nr = KF + L - k0 * L
                        abuf[0:nr, :] = rhs_jit(n, i, k0)
                        rhs = pltpu.bitcast(au[0:nr // 2, :], bf16)
                    elif i in held:
                        rhs = held[i]
                    elif pair and i in (1, 3):
                        rhs, held[i + 1] = rhs_pair(n, i, k0)
                    else:
                        rhs = rhs_jit(n, i, k0)
                    m[i] = jnp.dot(lhs_for(i, k0), rhs, preferred_element_type=f32)
                    if k0:
                        m[i] = m[i] + acc[i, :, n * L:(n + 1) * L]
                    fence(idx)
                return m

            def epilogue(n, m, split=None, start=True):
                j, t = _divmod_pow2(n, TPS)
                sc = sc_ref[...]
                sh = sh_ref[...]
                s12 = m[1] + m[2]
                d12 = m[1] - m[2]
                s34 = m[3] + m[4]
                d34 = m[3] - m[4]
                y0 = m[0] + s12 + s34
                p = A_ * d12
                q = B_ * d34
                y1 = p + q
                y2 = A2 * s12 + B2 * s34
                y3 = A2 * p + B2 * q + m[5]
                ys = (y0, y1, y2, y3)
                for p0, cnt in (split or ((0, 4),)):
                    for jj in range(p0, p0 + cnt):
                        h = ys[jj] * sc + sh
                        obuf[j, 4 * t + jj] = (h + h * jnp.tanh(h)).astype(bf16)
                    if not noout and start:
                        out_copy(n, p0, cnt).start()

            def kmajor(kc, comps):
                for i in comps:
                    rhs = jnp.concatenate(
                        [t_jit(n, i, kc * L, (kc + 1) * L) for n in range(P)], axis=1).astype(bf16)
                    r = jnp.dot(pltpu.bitcast(gu[5 * i + kc], bf16), rhs, preferred_element_type=f32)
                    acc[i] = r if kc == 0 else acc[i] + r
                    fence(i)

            comps = (0, 5, 1, 2, 3, 4)
            names = dict(w0=wc[0], w1=wc[1], w2=wc[2], w3=wc[3], w4=wc[4], xh=pre[0],
                         **{f'x{i}': cp for i, cp in enumerate(xa)})
            done = {kc: 0 for kc in range(KM)}
            for pi, (waits, work) in enumerate(plan):
              with scope(f'wait{pi}'):
                for nm in waits.split():
                    for cp in (vc if nm == 'v' else [names[nm]]):
                        cp.wait()
              with (scope(f'phase{pi}') if pi < len(plan) - 1 else contextlib.nullcontext()):
                for wk in work.split():
                    if wk[0] == 's':
                        setup(int(wk[1]))
                    elif wk == 'bn':
                        bn_consts()
                    elif wk[0] == 'm':
                        kc, cnt = int(wk[1]), int(wk[2])
                        kmajor(kc, comps[done[kc]:done[kc] + cnt])
                        done[kc] += cnt
            assert all(v == 6 for v in done.values())
            early = 'xh' in ' '.join(p[0] for p in plan)
            with contextlib.nullcontext():
              for n in range(P):
                m = matmuls(n, False, k0=KM, stage=0 if (early and n == P - 1) else None)
                if n == P - 1 and early:
                    abuf[...] = rhs_jit(P, order[0])
                epilogue(n, m, start=not defer)
            with scope('waitpre'):
              for cp in pre[1 if early else 0:]:
                cp.wait()
            if defer and not noout:
                out_copy(0, 0, 4 * P).start()
            if not early:
                abuf[...] = rhs_jit(P, order[0])

            def body(it, cc):
                c0 = P + it * NT
                nxt = window(c0 + NT + 1)
                if spu == 0:
                    for cp in nxt:
                        cp.start()
                for u in range(NT):
                    m = matmuls(c0 + u, u == 0, stage=stg[1] if (stg and u == NT - stg[0]) else None)
                    for cp in nxt[u * spu:(u + 1) * spu]:
                        cp.start()
                    if u == NT - 1:
                        if pin:
                            xu[0, 0, 0:8, :] = jnp.zeros((8, L), u32)
                        abuf[...] = rhs_jit(c0 + NT, order[0])
                    epilogue(c0 + u, m, lastsplit if u == NT - 1 else None)
                with scope('loopwait'):
                    for cp in nxt:
                        cp.wait()
                return cc

            lax.fori_loop(0, NIT if nit is None else nit, body, 0)
            if not noout:
                if nit is None:
                  with scope('outwait'):
                    pltpu.make_async_copy(obuf, obuf, out_sem).wait()
                else:
                    for n in range(P + nit * NT):
                        out_copy(0).wait()

        anyspec = pl.BlockSpec(memory_space=pl.ANY)
        out = pl.pallas_call(
            kernel,
            in_specs=[anyspec] * 6,
            out_specs=anyspec,
            out_shape=jax.ShapeDtypeStruct((S, C, Bn), x.dtype),
            scratch_shapes=[
                pltpu.VMEM((NJ, S + 2, C, L), bf16),
                pltpu.VMEM((NJ, S, C, L), bf16),
                pltpu.VMEM((3, C, C), bf16),
                *[pltpu.VMEM((C,), bf16)] * 4,
                pltpu.VMEM((30, C, L), bf16),
                pltpu.VMEM((KF + L, L), bf16),
                pltpu.VMEM((6, C, P * L), f32),
                pltpu.VMEM((C, L), f32),
                pltpu.VMEM((C, L), f32),
                pltpu.SMEM((1,), jnp.int32),
                pltpu.SemaphoreType.DMA((NSEM,)),
                pltpu.SemaphoreType.DMA((KM + 2,)),
                pltpu.SemaphoreType.DMA((NK + 1,)),
                pltpu.SemaphoreType.DMA((4,)),
                pltpu.SemaphoreType.DMA(()),
            ],
            compiler_params=pltpu.CompilerParams(
                vmem_limit_bytes=120 * 1024 * 1024,
                disable_bounds_checks=True,
                disable_semaphore_checks=nosc,
            ),
        )(xt, w, mean, var, g, b)
        return jnp.transpose(out, (2, 0, 1))
    return fn


@jax.jit
def pallas_standalone__batchnorm__sampling_kernel(x, w, mean, var, g, b):
    return build()(x, w, mean, var, g, b)
```

```python
import jax
import jax.numpy as jnp
from jax import lax
import jax.experimental.pallas as pl
import jax.experimental.pallas.tpu as pltpu

f32 = jnp.float32
bf16 = jnp.bfloat16
u32 = jnp.uint32

L = 128
PA = 2.0 / 3.0
PB = 1.5
A2 = PA * PA
B2 = PB * PB
S2 = A2 + B2
NA = 2 * A2 * (A2 - B2)
NB = 2 * B2 * (B2 - A2)

P = 4
NT = 6
KM = 2
ORDER = (1, 2, 3, 4, 5, 0)
COMPS = (0, 5, 1, 2, 3, 4)


def _divmod_pow2(x, n):
    if isinstance(x, int):
        return x // n, x % n
    return lax.shift_right_logical(x, n.bit_length() - 1), lax.bitwise_and(x, n - 1)


def _kernel(x_hbm, w_hbm, mean_hbm, var_hbm, g_hbm, b_hbm, o_hbm,
            xbuf, obuf, wbuf, vb0, vb1, vb2, vb3, gt, abuf, kbuf, acc, sc_ref, sh_ref, fence_ref,
            x_sem, p_sems, w_sems, v_sem, out_sem):
    S, C, B = x_hbm.shape
    NJ = B // L
    TPS = S // 4
    NK = C // L
    KF = NK * L
    NIT = (NJ * TPS - P) // NT
    PP = 4 * P + 1

    def lanes(j):
        return pl.ds(j * L if isinstance(j, int) else pl.multiple_of(j * L, L), L)

    def x_copy(j, p0, n, sem, r0=0, r1=C):
        return pltpu.make_async_copy(
            x_hbm.at[pl.ds(p0, n), pl.ds(r0, r1 - r0), lanes(j)],
            xbuf.at[j, pl.ds(p0 + 1, n), pl.ds(r0, r1 - r0), :], sem)

    def window(c):
        out = []
        for u, cnt in [(0, 1)] + [(u, 2) for u in range(1, NT - 1, 2)] + [(NT - 1, 1)]:
            j, t = _divmod_pow2(c + u, TPS)
            out.append(x_copy(_divmod_pow2(j, NJ)[1], 4 * t, 4 * cnt, x_sem))
        return out

    def window_wait():
        whole = xbuf.at[0, pl.ds(0, 4 * NT)]
        pltpu.make_async_copy(whole, whole, x_sem).wait()

    def out_copy(n, p0, cnt):
        j, t = _divmod_pow2(n, TPS)
        return pltpu.make_async_copy(
            obuf.at[j, pl.ds(4 * t + p0, cnt)], o_hbm.at[pl.ds(4 * t + p0, cnt), :, lanes(j)], out_sem)

    wc = [pltpu.make_async_copy(w_hbm.at[:, pl.ds(kc * L, min(L, C - kc * L)), :],
                                wbuf.at[:, pl.ds(kc * L, min(L, C - kc * L)), :], w_sems.at[kc])
          for kc in range(NK + 1)]
    vbuf = (vb0, vb1, vb2, vb3)
    vc = [pltpu.make_async_copy(r, vbuf[i], v_sem) for i, r in enumerate((mean_hbm, var_hbm, g_hbm, b_hbm))]
    xk = [x_copy(0, 0, PP, p_sems.at[kc], kc * L, (kc + 1) * L) for kc in range(KM)]
    xe = x_copy(0, 0, PP, p_sems.at[KM], KM * L, C)
    xh = x_copy(0, PP, 3, p_sems.at[KM + 1])

    for cp in [wc[0], *vc, xk[0], wc[1], xk[1], wc[2], wc[3], wc[4], xe, xh, *window(P + 1)]:
        cp.start()

    for j in range(NJ):
        xbuf[j, 0] = jnp.zeros((C, L), bf16)
        xbuf[j, S + 1] = jnp.zeros((C, L), bf16)

    def setup(kc):
        if kc < NK:
            blk = [wbuf[k, kc * L:(kc + 1) * L, :].astype(f32) for k in range(3)]
        else:
            r = [wbuf[k, KF:, :].astype(f32) for k in range(3)]
            z = jnp.zeros_like(r[0])
            blk = [jnp.concatenate([r[0], -r[0]], axis=0), jnp.concatenate([r[1], z], axis=0),
                   jnp.concatenate([r[2], z], axis=0)]
        w0, w1, w2 = (t.T for t in blk)
        ea = (w0 + A2 * w2) * (1.0 / NA)
        oa = w1 * (PA / NA)
        eb = (w0 + B2 * w2) * (1.0 / NB)
        ob = w1 * (PB / NB)
        for i, gi in enumerate([w0, ea + oa, ea - oa, eb + ob, eb - ob, w2]):
            if i > 0 or kc < NK:
                gt[5 * i + kc] = gi.astype(bf16)

    def bn_consts():
        mean, var, g, b = (r[...].astype(f32).reshape(1, C) for r in vbuf)
        sc = 0.5 * g * lax.rsqrt(var + 1e-5)
        sh = 0.5 * b - mean * sc
        sc_ref[...] = jnp.broadcast_to(sc, (L, C)).T
        sh_ref[...] = jnp.broadcast_to(sh, (L, C)).T

    gt_u = gt.bitcast(u32)
    abuf_u = abuf.bitcast(u32)
    kbuf_u = kbuf.bitcast(u32)

    def t_in(n, i, lo, hi):
        j, t = _divmod_pow2(n, TPS)
        j = _divmod_pow2(j, NJ)[1]
        d = lambda q: xbuf[j, 4 * t + q, lo:hi, :].astype(f32)
        if i == 0:
            return (d(0) + d(4)) - S2 * d(2)
        if i == 5:
            return (d(1) + d(5)) - S2 * d(3)
        c2, c1, c3 = {1: (B2, -PB, PA), 2: (B2, PB, -PA), 3: (A2, -PA, PB), 4: (A2, PA, -PB)}[i]
        return (d(4) - c2 * d(2)) + (c1 * d(1) + c3 * d(3))

    def rhs(n, i, k0=0):
        if i == 0:
            return t_in(n, 0, k0 * L, KF).astype(bf16)
        return jnp.concatenate([t_in(n, i, k0 * L, C), t_in(n, 0, KF, C)], axis=0).astype(bf16)

    def lhs(i, k0=0):
        return jnp.concatenate(
            [pltpu.bitcast(gt_u[5 * i + kc], bf16) for kc in range(k0, NK if i == 0 else NK + 1)], axis=1)

    def fence(v):
        fence_ref[0] = v

    def matmuls(n, first=None, k0=0):
        m = [None] * 6
        for idx, i in enumerate(ORDER):
            if idx == 0 and first:
                if first == 'stage':
                    abuf[...] = rhs(n, i)
                r = pltpu.bitcast(abuf_u[...], bf16)
            else:
                r = rhs(n, i, k0)
            m[i] = jnp.dot(lhs(i, k0), r, preferred_element_type=f32)
            if k0:
                m[i] = m[i] + acc[i, :, n * L:(n + 1) * L]
            fence(idx)
        return m

    def finish(n, m, groups):
        j, t = _divmod_pow2(n, TPS)
        sc = sc_ref[...]
        sh = sh_ref[...]
        s12 = m[1] + m[2]
        d12 = m[1] - m[2]
        s34 = m[3] + m[4]
        d34 = m[3] - m[4]
        p = PA * d12
        q = PB * d34
        y = (m[0] + s12 + s34, p + q, A2 * s12 + B2 * s34, A2 * p + B2 * q + m[5])
        for p0, cnt in groups or ((0, 4),):
            for s in range(p0, p0 + cnt):
                h = y[s] * sc + sh
                obuf[j, 4 * t + s] = (h + h * jnp.tanh(h)).astype(bf16)
            if groups:
                out_copy(n, p0, cnt).start()

    def chunk_dot(kc, i, staged=False):
        if staged:
            r = jnp.concatenate([pltpu.bitcast(kbuf_u[n], bf16) for n in range(P)], axis=1)
        else:
            r = jnp.concatenate([t_in(n, i, kc * L, (kc + 1) * L) for n in range(P)], axis=1).astype(bf16)
        r = jnp.dot(pltpu.bitcast(gt_u[5 * i + kc], bf16), r, preferred_element_type=f32)
        acc[i] = r if kc == 0 else acc[i] + r
        fence(i)

    def chunk_stage(kc, i):
        for n in range(P):
            kbuf[n] = t_in(n, i, kc * L, (kc + 1) * L).astype(bf16)

    wc[0].wait()
    for cp in vc:
        cp.wait()
    setup(0)
    bn_consts()

    xk[0].wait()
    for i in COMPS[:5]:
        chunk_dot(0, i)
    chunk_stage(0, COMPS[5])

    for cp in (wc[1], xk[1], wc[2]):
        cp.wait()
    chunk_dot(0, COMPS[5], staged=True)
    setup(1)
    setup(2)
    for i in COMPS[:3]:
        chunk_dot(1, i)
    chunk_stage(1, COMPS[3])

    for cp in (wc[3], wc[4]):
        cp.wait()
    chunk_dot(1, COMPS[3], staged=True)
    setup(3)
    setup(4)
    for i in COMPS[4:]:
        chunk_dot(1, i)

    xe.wait()
    for n in range(P):
        finish(n, matmuls(n, k0=KM), None)

    xh.wait()
    window_wait()
    out_copy(0, 0, 4 * P).start()
    abuf[...] = rhs(P, ORDER[0])

    def body(it, carry):
        c0 = P + it * NT
        for cp in window(c0 + NT + 1):
            cp.start()
        for u in range(NT):
            last = u == NT - 1
            m = matmuls(c0 + u, 'carried' if u == 0 else 'stage' if last else None)
            if last:
                abuf[...] = rhs(c0 + NT, ORDER[0])
            finish(c0 + u, m, ((1, 2), (3, 1), (0, 1)) if last else ((0, 4),))
        window_wait()
        return carry

    lax.fori_loop(0, NIT, body, 0)
    pltpu.make_async_copy(obuf, obuf, out_sem).wait()


@jax.jit
def pallas_standalone__batchnorm__sampling_kernel(x, w, mean, var, g, b):
    B, S, C = x.shape
    NJ = B // L
    NK = C // L
    assert w.shape == (3, C, C) and C == NK * L + L // 2 and S == 32 and NJ == 8 and NK == 4
    hbm = pl.BlockSpec(memory_space=pl.ANY)
    out = pl.pallas_call(
        _kernel,
        in_specs=[hbm] * 6,
        out_specs=hbm,
        out_shape=jax.ShapeDtypeStruct((S, C, B), x.dtype),
        scratch_shapes=[
            pltpu.VMEM((NJ, S + 2, C, L), bf16),
            pltpu.VMEM((NJ, S, C, L), bf16),
            pltpu.VMEM((3, C, C), bf16),
            *[pltpu.VMEM((C,), bf16)] * 4,
            pltpu.VMEM((6 * (NK + 1), C, L), bf16),
            pltpu.VMEM(((NK + 1) * L, L), bf16),
            pltpu.VMEM((P, L, L), bf16),
            pltpu.VMEM((6, C, P * L), f32),
            pltpu.VMEM((C, L), f32),
            pltpu.VMEM((C, L), f32),
            pltpu.SMEM((1,), jnp.int32),
            pltpu.SemaphoreType.DMA(()),
            pltpu.SemaphoreType.DMA((KM + 2,)),
            pltpu.SemaphoreType.DMA((NK + 1,)),
            pltpu.SemaphoreType.DMA(()),
            pltpu.SemaphoreType.DMA(()),
        ],
        compiler_params=pltpu.CompilerParams(
            vmem_limit_bytes=120 * 1024 * 1024,
            disable_bounds_checks=True,
            disable_semaphore_checks=True,
        ),
    )(jnp.transpose(x, (1, 2, 0)), w, mean, var, g, b)
    return jnp.transpose(out, (2, 0, 1))
```

```python
import jax
import jax.numpy as jnp
from jax import lax
import jax.experimental.pallas as pl
import jax.experimental.pallas.tpu as pltpu

f32 = jnp.float32
bf16 = jnp.bfloat16
u32 = jnp.uint32

L = 128
PA = 2.0 / 3.0
PB = 1.5
A2 = PA * PA
B2 = PB * PB
S2 = A2 + B2
NA = 2 * A2 * (A2 - B2)
NB = 2 * B2 * (B2 - A2)

P = 4
NT = 6
KM = 2
ORDER = (1, 2, 3, 4, 5, 0)
COMPS = (0, 5, 1, 2, 3, 4)


def _divmod_pow2(x, n):
    if isinstance(x, int):
        return x // n, x % n
    return lax.shift_right_logical(x, n.bit_length() - 1), lax.bitwise_and(x, n - 1)


def _kernel(x_hbm, w_hbm, mean_hbm, var_hbm, g_hbm, b_hbm, o_hbm,
            xbuf, obuf, wbuf, vb0, vb1, vb2, vb3, gt, abuf, kbuf, acc, sc_ref, sh_ref, fence_ref,
            x_sems, p_sems, w_sems, v_sem, out_sem):
    S, C, B = x_hbm.shape
    NJ = B // L
    TPS = S // 4
    NK = C // L
    KF = NK * L
    NIT = (NJ * TPS - P) // NT
    PP = 4 * P + 1

    def lanes(j):
        return pl.ds(j * L if isinstance(j, int) else pl.multiple_of(j * L, L), L)

    def x_copy(j, p0, n, sem, r0=0, r1=C):
        return pltpu.make_async_copy(
            x_hbm.at[pl.ds(p0, n), pl.ds(r0, r1 - r0), lanes(j)],
            xbuf.at[j, pl.ds(p0 + 1, n), pl.ds(r0, r1 - r0), :], sem)

    def window(c):
        out = []
        for u, cnt in [(0, 1)] + [(u, 2) for u in range(1, NT - 1, 2)] + [(NT - 1, 1)]:
            j, t = _divmod_pow2(c + u, TPS)
            out.append(x_copy(_divmod_pow2(j, NJ)[1], 4 * t, 4 * cnt, x_sems.at[len(out)]))
        return out

    def out_copy(n, p0, cnt):
        j, t = _divmod_pow2(n, TPS)
        return pltpu.make_async_copy(
            obuf.at[j, pl.ds(4 * t + p0, cnt)], o_hbm.at[pl.ds(4 * t + p0, cnt), :, lanes(j)], out_sem)

    wc = [pltpu.make_async_copy(w_hbm.at[:, pl.ds(kc * L, min(L, C - kc * L)), :],
                                wbuf.at[:, pl.ds(kc * L, min(L, C - kc * L)), :], w_sems.at[kc])
          for kc in range(NK + 1)]
    vbuf = (vb0, vb1, vb2, vb3)
    vc = [pltpu.make_async_copy(r, vbuf[i], v_sem) for i, r in enumerate((mean_hbm, var_hbm, g_hbm, b_hbm))]
    xk = [x_copy(0, 0, PP, p_sems.at[kc], kc * L, (kc + 1) * L) for kc in range(KM)]
    xe = x_copy(0, 0, PP, p_sems.at[KM], KM * L, C)
    xh = x_copy(0, PP, 3, p_sems.at[KM + 1])

    first = window(P + 1)

    for cp in [wc[0], *vc, xk[0], wc[1], xk[1], wc[2], wc[3], wc[4], xe, xh, *first]:
        cp.start()

    for j in range(NJ):
        xbuf[j, 0] = jnp.zeros((C, L), bf16)
        xbuf[j, S + 1] = jnp.zeros((C, L), bf16)

    def setup(kc):
        if kc < NK:
            blk = [wbuf[k, kc * L:(kc + 1) * L, :].astype(f32) for k in range(3)]
        else:
            r = [wbuf[k, KF:, :].astype(f32) for k in range(3)]
            z = jnp.zeros_like(r[0])
            blk = [jnp.concatenate([r[0], -r[0]], axis=0), jnp.concatenate([r[1], z], axis=0),
                   jnp.concatenate([r[2], z], axis=0)]
        w0, w1, w2 = (t.T for t in blk)
        ea = (w0 + A2 * w2) * (1.0 / NA)
        oa = w1 * (PA / NA)
        eb = (w0 + B2 * w2) * (1.0 / NB)
        ob = w1 * (PB / NB)
        for i, gi in enumerate([w0, ea + oa, ea - oa, eb + ob, eb - ob, w2]):
            if i > 0 or kc < NK:
                gt[5 * i + kc] = pltpu.bitcast(gi.astype(bf16), u32)

    def bn_consts():
        mean, var, g, b = (r[...].astype(f32).reshape(1, C) for r in vbuf)
        sc = 0.5 * g * lax.rsqrt(var + 1e-5)
        sh = 0.5 * b - mean * sc
        sc_ref[...] = jnp.broadcast_to(sc, (L, C)).T
        sh_ref[...] = jnp.broadcast_to(sh, (L, C)).T

    def t_in(n, i, lo, hi):
        j, t = _divmod_pow2(n, TPS)
        j = _divmod_pow2(j, NJ)[1]
        d = lambda q: xbuf[j, 4 * t + q, lo:hi, :].astype(f32)
        if i == 0:
            return (d(0) + d(4)) - S2 * d(2)
        if i == 5:
            return (d(1) + d(5)) - S2 * d(3)
        c2, c1, c3 = {1: (B2, -PB, PA), 2: (B2, PB, -PA), 3: (A2, -PA, PB), 4: (A2, PA, -PB)}[i]
        return (d(4) - c2 * d(2)) + (c1 * d(1) + c3 * d(3))

    def rhs(n, i, k0=0):
        if i == 0:
            return t_in(n, 0, k0 * L, KF).astype(bf16)
        return jnp.concatenate([t_in(n, i, k0 * L, C), t_in(n, 0, KF, C)], axis=0).astype(bf16)

    def lhs(i, k0=0):
        return jnp.concatenate(
            [pltpu.bitcast(gt[5 * i + kc], bf16) for kc in range(k0, NK if i == 0 else NK + 1)], axis=1)

    def fence(v):
        fence_ref[0] = v

    def matmuls(n, first=None, k0=0):
        m = [None] * 6
        for idx, i in enumerate(ORDER):
            if idx == 0 and first:
                if first == 'stage':
                    abuf[...] = pltpu.bitcast(rhs(n, i), u32)
                r = pltpu.bitcast(abuf[...], bf16)
            else:
                r = rhs(n, i, k0)
            m[i] = jnp.dot(lhs(i, k0), r, preferred_element_type=f32)
            if k0:
                m[i] = m[i] + acc[i, :, n * L:(n + 1) * L]
            fence(idx)
        return m

    def finish(n, m, groups):
        j, t = _divmod_pow2(n, TPS)
        sc = sc_ref[...]
        sh = sh_ref[...]
        s12 = m[1] + m[2]
        d12 = m[1] - m[2]
        s34 = m[3] + m[4]
        d34 = m[3] - m[4]
        p = PA * d12
        q = PB * d34
        y = (m[0] + s12 + s34, p + q, A2 * s12 + B2 * s34, A2 * p + B2 * q + m[5])
        for p0, cnt in groups or ((0, 4),):
            for s in range(p0, p0 + cnt):
                h = y[s] * sc + sh
                obuf[j, 4 * t + s] = (h + h * jnp.tanh(h)).astype(bf16)
            if groups:
                out_copy(n, p0, cnt).start()

    def chunk_dot(kc, i, staged=False):
        if staged:
            r = jnp.concatenate([pltpu.bitcast(kbuf[n], bf16) for n in range(P)], axis=1)
        else:
            r = jnp.concatenate([t_in(n, i, kc * L, (kc + 1) * L) for n in range(P)], axis=1).astype(bf16)
        r = jnp.dot(pltpu.bitcast(gt[5 * i + kc], bf16), r, preferred_element_type=f32)
        acc[i] = r if kc == 0 else acc[i] + r
        fence(i)

    def chunk_stage(kc, i):
        for n in range(P):
            kbuf[n] = pltpu.bitcast(t_in(n, i, kc * L, (kc + 1) * L).astype(bf16), u32)

    wc[0].wait()
    for cp in vc:
        cp.wait()
    setup(0)
    bn_consts()

    xk[0].wait()
    for i in COMPS[:5]:
        chunk_dot(0, i)
    chunk_stage(0, COMPS[5])

    for cp in (wc[1], xk[1], wc[2]):
        cp.wait()
    chunk_dot(0, COMPS[5], staged=True)
    setup(1)
    setup(2)
    for i in COMPS[:3]:
        chunk_dot(1, i)
    chunk_stage(1, COMPS[3])

    for cp in (wc[3], wc[4]):
        cp.wait()
    chunk_dot(1, COMPS[3], staged=True)
    setup(3)
    setup(4)
    for i in COMPS[4:]:
        chunk_dot(1, i)

    xe.wait()
    for n in range(P):
        finish(n, matmuls(n, k0=KM), None)

    for cp in (xh, *first):
        cp.wait()
    out_copy(0, 0, 4 * P).start()
    abuf[...] = pltpu.bitcast(rhs(P, ORDER[0]), u32)

    def body(it, carry):
        c0 = P + it * NT
        nxt = window(c0 + NT + 1)
        for cp in nxt:
            cp.start()
        for u in range(NT):
            last = u == NT - 1
            m = matmuls(c0 + u, 'carried' if u == 0 else 'stage' if last else None)
            if last:
                abuf[...] = pltpu.bitcast(rhs(c0 + NT, ORDER[0]), u32)
            finish(c0 + u, m, ((1, 2), (3, 1), (0, 1)) if last else ((0, 4),))
        for cp in nxt:
            cp.wait()
        return carry

    lax.fori_loop(0, NIT, body, 0)
    pltpu.make_async_copy(o_hbm, o_hbm, out_sem).wait()


@jax.jit
def pallas_standalone__batchnorm__sampling_kernel(x, w, mean, var, g, b):
    B, S, C = x.shape
    NJ = B // L
    NK = C // L
    assert w.shape == (3, C, C) and C == NK * L + L // 2 and S == 32 and NJ == 8 and NK == 4
    hbm = pl.BlockSpec(memory_space=pl.ANY)
    out = pl.pallas_call(
        _kernel,
        in_specs=[hbm] * 6,
        out_specs=hbm,
        out_shape=jax.ShapeDtypeStruct((S, C, B), x.dtype),
        scratch_shapes=[
            pltpu.VMEM((NJ, S + 2, C, L), bf16),
            pltpu.VMEM((NJ, S, C, L), bf16),
            pltpu.VMEM((3, C, C), bf16),
            *[pltpu.VMEM((C,), bf16)] * 4,
            pltpu.VMEM((6 * (NK + 1), C // 2, L), u32),
            pltpu.VMEM(((NK + 1) * L // 2, L), u32),
            pltpu.VMEM((P, L // 2, L), u32),
            pltpu.VMEM((6, C, P * L), f32),
            pltpu.VMEM((C, L), f32),
            pltpu.VMEM((C, L), f32),
            pltpu.SMEM((1,), jnp.int32),
            pltpu.SemaphoreType.DMA((NT // 2 + 1,)),
            pltpu.SemaphoreType.DMA((KM + 2,)),
            pltpu.SemaphoreType.DMA((NK + 1,)),
            pltpu.SemaphoreType.DMA(()),
            pltpu.SemaphoreType.DMA(()),
        ],
        compiler_params=pltpu.CompilerParams(
            vmem_limit_bytes=120 * 1024 * 1024,
            disable_bounds_checks=True,
            disable_semaphore_checks=True,
        ),
    )(jnp.transpose(x, (1, 2, 0)), w, mean, var, g, b)
    return jnp.transpose(out, (2, 0, 1))
```

```python
import jax
import jax.numpy as jnp
from jax import lax
import jax.experimental.pallas as pl
import jax.experimental.pallas.tpu as pltpu

f32 = jnp.float32
bf16 = jnp.bfloat16
u32 = jnp.uint32

L = 128
PA = 2.0 / 3.0
PB = 1.5
A2 = PA * PA
B2 = PB * PB
S2 = A2 + B2
NA = 2 * A2 * (A2 - B2)
NB = 2 * B2 * (B2 - A2)

P = 4
NT = 6
KM = 2
ORDER = (1, 2, 3, 4, 5, 0)
COMPS = (0, 5, 1, 2, 3, 4)


def _divmod_pow2(x, n):
    if isinstance(x, int):
        return x // n, x % n
    return lax.shift_right_logical(x, n.bit_length() - 1), lax.bitwise_and(x, n - 1)


def _kernel(x_hbm, w_hbm, mean_hbm, var_hbm, g_hbm, b_hbm, o_hbm,
            xbuf, obuf, wbuf, vb0, vb1, vb2, vb3, gnew, gt, abuf, kbuf, acc, sc_ref, sh_ref, fence_ref,
            x_sem, p_sems, w_sems, v_sem, out_sem):
    S, C, B = x_hbm.shape
    NJ = B // L
    TPS = S // 4
    NK = C // L
    KF = NK * L
    NIT = (NJ * TPS - P) // NT
    PP = 4 * P + 1

    def lanes(j):
        return pl.ds(j * L if isinstance(j, int) else pl.multiple_of(j * L, L), L)

    def x_copy(j, p0, n, sem, r0=0, r1=C):
        return pltpu.make_async_copy(
            x_hbm.at[pl.ds(p0, n), pl.ds(r0, r1 - r0), lanes(j)],
            xbuf.at[j, pl.ds(p0 + 1, n), pl.ds(r0, r1 - r0), :], sem)

    def window(c):
        out = []
        for u, cnt in [(0, 1)] + [(u, 2) for u in range(1, NT - 1, 2)] + [(NT - 1, 1)]:
            j, t = _divmod_pow2(c + u, TPS)
            out.append(x_copy(_divmod_pow2(j, NJ)[1], 4 * t, 4 * cnt, x_sem))
        return out

    def window_wait():
        total = xbuf.at[0, pl.ds(0, 4 * NT)]
        pltpu.make_async_copy(total, total, x_sem).wait()

    def out_copy(n, p0, cnt):
        j, t = _divmod_pow2(n, TPS)
        return pltpu.make_async_copy(
            obuf.at[j, pl.ds(4 * t + p0, cnt)], o_hbm.at[pl.ds(4 * t + p0, cnt), :, lanes(j)], out_sem)

    wc = [pltpu.make_async_copy(w_hbm.at[:, pl.ds(kc * L, min(L, C - kc * L)), :],
                                wbuf.at[:, pl.ds(kc * L, min(L, C - kc * L)), :], w_sems.at[kc])
          for kc in range(NK + 1)]
    vbuf = (vb0, vb1, vb2, vb3)
    vc = [pltpu.make_async_copy(r, vbuf[i], v_sem) for i, r in enumerate((mean_hbm, var_hbm, g_hbm, b_hbm))]
    xk = [x_copy(0, 0, PP, p_sems.at[kc], kc * L, (kc + 1) * L) for kc in range(KM)]
    xe = x_copy(0, 0, PP, p_sems.at[KM], KM * L, C)
    xh = x_copy(0, PP, 3, p_sems.at[KM + 1])

    for cp in [wc[0], *vc, xk[0], wc[1], xk[1], wc[2], wc[3], wc[4], xe, xh, *window(P + 1)]:
        cp.start()

    for j in range(NJ):
        xbuf[j, 0] = jnp.zeros((C, L), bf16)
        xbuf[j, S + 1] = jnp.zeros((C, L), bf16)

    def setup(kc):
        if kc < NK:
            blk = [wbuf[k, kc * L:(kc + 1) * L, :].astype(f32) for k in range(3)]
        else:
            r = [wbuf[k, KF:, :].astype(f32) for k in range(3)]
            z = jnp.zeros_like(r[0])
            blk = [jnp.concatenate([r[0], -r[0]], axis=0), jnp.concatenate([r[1], z], axis=0),
                   jnp.concatenate([r[2], z], axis=0)]
        w0, w1, w2 = (t.T for t in blk)
        ea = (w0 + A2 * w2) * (1.0 / NA)
        oa = w1 * (PA / NA)
        eb = (w0 + B2 * w2) * (1.0 / NB)
        ob = w1 * (PB / NB)
        for i, gi in enumerate([w0, ea + oa, ea - oa, eb + ob, eb - ob, w2]):
            if i > 0 or kc < NK:
                gnew[5 * i + kc] = gi.astype(bf16)

    def bn_consts():
        mean, var, g, b = (r[...].astype(f32).reshape(1, C) for r in vbuf)
        sc = 0.5 * g * lax.rsqrt(var + 1e-5)
        sh = 0.5 * b - mean * sc
        sc_ref[...] = jnp.broadcast_to(sc, (L, C)).T
        sh_ref[...] = jnp.broadcast_to(sh, (L, C)).T

    def t_in(n, i, lo, hi):
        j, t = _divmod_pow2(n, TPS)
        j = _divmod_pow2(j, NJ)[1]
        d = lambda q: xbuf[j, 4 * t + q, lo:hi, :].astype(f32)
        if i == 0:
            return (d(0) + d(4)) - S2 * d(2)
        if i == 5:
            return (d(1) + d(5)) - S2 * d(3)
        c2, c1, c3 = {1: (B2, -PB, PA), 2: (B2, PB, -PA), 3: (A2, -PA, PB), 4: (A2, PA, -PB)}[i]
        return (d(4) - c2 * d(2)) + (c1 * d(1) + c3 * d(3))

    def rhs(n, i, k0=0):
        if i == 0:
            return t_in(n, 0, k0 * L, KF)
        return jnp.concatenate([t_in(n, i, k0 * L, C), t_in(n, 0, KF, C)], axis=0)

    def g_tile(col, fresh):
        if not fresh:
            return pltpu.bitcast(gt[col], bf16)
        v = gnew[col]
        gt[col] = pltpu.bitcast(v, u32)
        return v

    def lhs(i, k0=0, fresh=False):
        return jnp.concatenate(
            [g_tile(5 * i + kc, fresh) for kc in range(k0, NK if i == 0 else NK + 1)], axis=1)

    def fence(v):
        fence_ref[0] = v

    def matmuls(n, first=None, k0=0):
        m = [None] * 6
        for idx, i in enumerate(ORDER):
            if idx == 0 and first:
                if first == 'stage':
                    abuf[...] = rhs(n, i)
                r = abuf[...]
            else:
                r = rhs(n, i, k0)
            m[i] = jnp.dot(lhs(i, k0, fresh=(k0 > 0 and n == 0)), r.astype(bf16), preferred_element_type=f32)
            if k0:
                m[i] = m[i] + acc[i, :, n * L:(n + 1) * L]
            fence(idx)
        return m

    def finish(n, m, groups):
        j, t = _divmod_pow2(n, TPS)
        sc = sc_ref[...]
        sh = sh_ref[...]
        s12 = m[1] + m[2]
        d12 = m[1] - m[2]
        s34 = m[3] + m[4]
        d34 = m[3] - m[4]
        p = PA * d12
        q = PB * d34
        y = (m[0] + s12 + s34, p + q, A2 * s12 + B2 * s34, A2 * p + B2 * q + m[5])
        for p0, cnt in groups or ((0, 4),):
            for s in range(p0, p0 + cnt):
                h = y[s] * sc + sh
                obuf[j, 4 * t + s] = (h + h * jnp.tanh(h)).astype(bf16)
            if groups:
                out_copy(n, p0, cnt).start()

    def chunk_dot(kc, i, staged=False):
        if staged:
            r = jnp.concatenate([kbuf[n] for n in range(P)], axis=1).astype(bf16)
        else:
            r = jnp.concatenate([t_in(n, i, kc * L, (kc + 1) * L) for n in range(P)], axis=1).astype(bf16)
        r = jnp.dot(g_tile(5 * i + kc, True), r, preferred_element_type=f32)
        acc[i] = r if kc == 0 else acc[i] + r
        fence(i)

    def chunk_stage(kc, i):
        for n in range(P):
            kbuf[n] = t_in(n, i, kc * L, (kc + 1) * L)

    wc[0].wait()
    for cp in vc:
        cp.wait()
    setup(0)
    bn_consts()

    xk[0].wait()
    for i in COMPS[:5]:
        chunk_dot(0, i)
    chunk_stage(0, COMPS[5])

    for cp in (wc[1], xk[1], wc[2]):
        cp.wait()
    chunk_dot(0, COMPS[5], staged=True)
    setup(1)
    setup(2)
    for i in COMPS[:3]:
        chunk_dot(1, i)
    chunk_stage(1, COMPS[3])

    for cp in (wc[3], wc[4]):
        cp.wait()
    chunk_dot(1, COMPS[3], staged=True)
    setup(3)
    setup(4)
    for i in COMPS[4:]:
        chunk_dot(1, i)

    xe.wait()
    for n in range(P):
        finish(n, matmuls(n, k0=KM), None)

    xh.wait()
    window_wait()
    out_copy(0, 0, 4 * P).start()
    abuf[...] = rhs(P, ORDER[0])

    def body(it, carry):
        c0 = P + it * NT
        for cp in window(c0 + NT + 1):
            cp.start()
        for u in range(NT):
            last = u == NT - 1
            m = matmuls(c0 + u, 'carried' if u == 0 else 'stage' if last else None)
            if last:
                abuf[...] = rhs(c0 + NT, ORDER[0])
            finish(c0 + u, m, ((1, 2), (3, 1), (0, 1)) if last else ((0, 4),))
        window_wait()
        return carry

    lax.fori_loop(0, NIT, body, 0)
    pltpu.make_async_copy(o_hbm, o_hbm, out_sem).wait()


@jax.jit
def pallas_standalone__batchnorm__sampling_kernel(x, w, mean, var, g, b):
    B, S, C = x.shape
    NJ = B // L
    NK = C // L
    assert w.shape == (3, C, C) and C == NK * L + L // 2 and S == 32 and NJ == 8 and NK == 4
    hbm = pl.BlockSpec(memory_space=pl.ANY)
    out = pl.pallas_call(
        _kernel,
        in_specs=[hbm] * 6,
        out_specs=hbm,
        out_shape=jax.ShapeDtypeStruct((S, C, B), x.dtype),
        scratch_shapes=[
            pltpu.VMEM((NJ, S + 2, C, L), bf16),
            pltpu.VMEM((NJ, S, C, L), bf16),
            pltpu.VMEM((3, C, C), bf16),
            *[pltpu.VMEM((C,), bf16)] * 4,
            pltpu.VMEM((6 * (NK + 1), C, L), bf16),
            pltpu.VMEM((6 * (NK + 1), C // 2, L), u32),
            pltpu.VMEM(((NK + 1) * L, L), f32),
            pltpu.VMEM((P, L, L), f32),
            pltpu.VMEM((6, C, P * L), f32),
            pltpu.VMEM((C, L), f32),
            pltpu.VMEM((C, L), f32),
            pltpu.SMEM((1,), jnp.int32),
            pltpu.SemaphoreType.DMA(()),
            pltpu.SemaphoreType.DMA((KM + 2,)),
            pltpu.SemaphoreType.DMA((NK + 1,)),
            pltpu.SemaphoreType.DMA(()),
            pltpu.SemaphoreType.DMA(()),
        ],
        compiler_params=pltpu.CompilerParams(
            vmem_limit_bytes=120 * 1024 * 1024,
            disable_bounds_checks=True,
            disable_semaphore_checks=True,
        ),
    )(jnp.transpose(x, (1, 2, 0)), w, mean, var, g, b)
    return jnp.transpose(out, (2, 0, 1))
```

```python
import jax
import jax.numpy as jnp
from jax import lax
import jax.experimental.pallas as pl
import jax.experimental.pallas.tpu as pltpu

f32 = jnp.float32
bf16 = jnp.bfloat16
u32 = jnp.uint32

L = 128
PA = 2.0 / 3.0
PB = 1.5
A2 = PA * PA
B2 = PB * PB
S2 = A2 + B2
NA = 2 * A2 * (A2 - B2)
NB = 2 * B2 * (B2 - A2)

P = 4
NT = 6
ORDER = (1, 2, 3, 4, 5, 0)
COMPS = (0, 5, 1, 2, 3, 4)


def _divmod_pow2(x, n):
    if isinstance(x, int):
        return x // n, x % n
    return lax.shift_right_logical(x, n.bit_length() - 1), lax.bitwise_and(x, n - 1)


def _dot(a, b):
    return jnp.dot(a, b.astype(bf16), preferred_element_type=f32)


def _kernel(x_hbm, w_hbm, mean_hbm, var_hbm, g_hbm, b_hbm, o_hbm,
            xbuf, obuf, wbuf, vb0, vb1, vb2, vb3, gnew, gt, abuf, acc, sc_ref, sh_ref, fence_ref,
            x_sem, p_sems, w_sems, v_sem, out_sem):
    S, C, B = x_hbm.shape
    NJ = B // L
    TPS = S // 4
    NK = C // L
    KF = NK * L
    H = C // 2
    NIT = (NJ * TPS - P) // NT
    PP = 4 * P + 1
    SHARED = 6 * (NK + 1) - 1

    def lanes(j):
        return pl.ds(j * L if isinstance(j, int) else pl.multiple_of(j * L, L), L)

    def x_copy(j, p0, n, sem, r0=0, r1=C):
        return pltpu.make_async_copy(
            x_hbm.at[pl.ds(p0, n), pl.ds(r0, r1 - r0), lanes(j)],
            xbuf.at[j, pl.ds(p0 + 1, n), pl.ds(r0, r1 - r0), :], sem)

    def window(c):
        out = []
        for u, cnt in [(0, 1)] + [(u, 2) for u in range(1, NT - 1, 2)] + [(NT - 1, 1)]:
            j, t = _divmod_pow2(c + u, TPS)
            out.append(x_copy(_divmod_pow2(j, NJ)[1], 4 * t, 4 * cnt, x_sem))
        return out

    def window_wait():
        total = xbuf.at[0, pl.ds(0, 4 * NT)]
        pltpu.make_async_copy(total, total, x_sem).wait()

    def out_copy(n, p0, cnt):
        j, t = _divmod_pow2(n, TPS)
        return pltpu.make_async_copy(
            obuf.at[j, pl.ds(4 * t + p0, cnt)], o_hbm.at[pl.ds(4 * t + p0, cnt), :, lanes(j)], out_sem)

    wc = [pltpu.make_async_copy(w_hbm.at[:, pl.ds(kc * L, min(L, C - kc * L)), :],
                                wbuf.at[:, pl.ds(kc * L, min(L, C - kc * L)), :], w_sems.at[kc])
          for kc in range(NK + 1)]
    vbuf = (vb0, vb1, vb2, vb3)
    vc = [pltpu.make_async_copy(r, vbuf[i], v_sem) for i, r in enumerate((mean_hbm, var_hbm, g_hbm, b_hbm))]
    x0, x1, xe, xr = (x_copy(0, 0, PP, p_sems.at[i], r0, r1)
                      for i, (r0, r1) in enumerate(((0, L), (L, 2 * L), (2 * L, KF), (KF, C))))
    xh = x_copy(0, PP, 3, p_sems.at[4])

    for cp in [wc[0], *vc, x0, wc[1], x1, wc[4], xr, wc[2], wc[3], xe, xh, *window(P + 1)]:
        cp.start()

    for j in range(NJ):
        xbuf[j, 0] = jnp.zeros((C, L), bf16)
        xbuf[j, S + 1] = jnp.zeros((C, L), bf16)

    def setup(kc):
        if kc < NK:
            w0, w1, w2 = (wbuf[k, kc * L:(kc + 1) * L, :].astype(f32).T for k in range(3))
        else:
            r = [wbuf[k, KF:, :].astype(f32) for k in range(3)]
            t0, t1, t2 = (jnp.concatenate(p, axis=0).T for p in ((r[0], -r[0]), (r[1], r[0]), (r[2], r[2])))
            left = lax.broadcasted_iota(jnp.int32, (H, L), 1) < L // 2
            w0 = jnp.concatenate([t0[:H], jnp.where(left, t0[H:], t2[:H])], axis=0)
            w1 = jnp.concatenate([jnp.where(left, t1[:H], t0[H:]), jnp.where(left, t1[H:], t2[H:])], axis=0)
            w2 = jnp.concatenate([jnp.where(left, t2[:H], 0.0), jnp.where(left, t2[H:], 0.0)], axis=0)
            gnew[SHARED, :H, :] = jnp.where(left, t2[:H], t1[H:]).astype(bf16)
        ea = (w0 + A2 * w2) * (1.0 / NA)
        oa = w1 * (PA / NA)
        eb = (w0 + B2 * w2) * (1.0 / NB)
        ob = w1 * (PB / NB)
        for i, gi in enumerate([w0, ea + oa, ea - oa, eb + ob, eb - ob, w2]):
            if kc < NK or 0 < i < 5:
                gnew[5 * i + kc] = gi.astype(bf16)

    def bn_consts():
        mean, var, g, b = (r[...].astype(f32).reshape(1, C) for r in vbuf)
        sc = 0.5 * g * lax.rsqrt(var + 1e-5)
        sh = 0.5 * b - mean * sc
        sc_ref[...] = jnp.broadcast_to(sc, (L, C)).T
        sh_ref[...] = jnp.broadcast_to(sh, (L, C)).T

    def t_in(n, i, lo, hi):
        j, t = _divmod_pow2(n, TPS)
        j = _divmod_pow2(j, NJ)[1]
        d = lambda q: xbuf[j, 4 * t + q, lo:hi, :].astype(f32)
        if i == 0:
            return (d(0) + d(4)) - S2 * d(2)
        if i == 5:
            return (d(1) + d(5)) - S2 * d(3)
        c2, c1, c3 = {1: (B2, -PB, PA), 2: (B2, PB, -PA), 3: (A2, -PA, PB), 4: (A2, PA, -PB)}[i]
        return (d(4) - c2 * d(2)) + (c1 * d(1) + c3 * d(3))

    def rem(n, i, k):
        return jnp.concatenate([t_in(n, i, KF, C), t_in(n, k, KF, C)], axis=0)

    def g_tiles(slots, fresh=False, lo=0, hi=C):
        out = []
        for slot in slots:
            if fresh:
                v = gnew[slot, lo:hi, :]
                gt[slot, lo // 2:hi // 2, :] = pltpu.bitcast(v, u32)
            else:
                v = pltpu.bitcast(gt[slot, lo // 2:hi // 2, :], bf16)
            out.append(v)
        return jnp.concatenate(out, axis=1)

    def fence(v):
        fence_ref[0] = v

    def stage(n, i):
        abuf[:KF, :] = t_in(n, i, 0, KF)
        abuf[KF:, :] = rem(n, i, 0)

    def matmuls(n, staged=None, restage=False):
        m = [None] * 6
        for idx, i in enumerate(ORDER):
            if 0 < i < 5:
                if idx == staged:
                    if restage:
                        stage(n, i)
                    main, top = abuf[:KF, :], abuf[KF:, :]
                else:
                    main, top = t_in(n, i, 0, KF), rem(n, i, 0)
                slots = range(5 * i, 5 * i + NK + 1)
                halves = [_dot(g_tiles(slots, lo=0, hi=H), jnp.concatenate([main, top], axis=0)),
                          _dot(g_tiles(slots, lo=H, hi=C), jnp.concatenate([main, rem(n, i, 5)], axis=0))]
            else:
                mi = _dot(g_tiles(range(5 * i, 5 * i + NK)), t_in(n, i, 0, KF))
                if i == 5:
                    shared = _dot(g_tiles([SHARED], lo=0, hi=H), rem(n, 5, 0))
                halves = [mi[:H] + shared, mi[H:]] if i == 5 else [mi[:H], mi[H:] + shared]
            m[i] = jnp.concatenate(halves, axis=0)
            fence(idx)
        return m

    def finish(n, m, groups):
        j, t = _divmod_pow2(n, TPS)
        sc = sc_ref[...]
        sh = sh_ref[...]
        s12 = m[1] + m[2]
        d12 = m[1] - m[2]
        s34 = m[3] + m[4]
        d34 = m[3] - m[4]
        p = PA * d12
        q = PB * d34
        y = (m[0] + s12 + s34, p + q, A2 * s12 + B2 * s34, A2 * p + B2 * q + m[5])
        for p0, cnt in groups or ((0, 4),):
            for s in range(p0, p0 + cnt):
                h = y[s] * sc + sh
                obuf[j, 4 * t + s] = (h + h * jnp.tanh(h)).astype(bf16)
            if groups:
                out_copy(n, p0, cnt).start()

    def chunk_dot(kc, i):
        r = _dot(g_tiles([5 * i + kc], fresh=True),
                 jnp.concatenate([t_in(n, i, kc * L, (kc + 1) * L) for n in range(P)], axis=1))
        acc[i] = r if kc == 0 else acc[i] + r
        fence(i)

    def rem_dot(i, k):
        lo = 0 if k == 0 else H
        r = _dot(g_tiles([SHARED if i == 5 else 5 * i + NK], fresh=True, lo=lo, hi=lo + H),
                 jnp.concatenate([rem(n, i, k) for n in range(P)], axis=1))
        acc[i, lo:lo + H, :] += r
        if i == 5:
            acc[0, H:, :] += r
        fence(i)

    rems = [(5, 0)] + [(i, k) for i in range(1, 5) for k in (0, 5)]

    for cp in (wc[0], *vc):
        cp.wait()
    setup(0)
    bn_consts()

    x0.wait()
    for i in COMPS[:4]:
        chunk_dot(0, i)

    for cp in (wc[1], x1, wc[4]):
        cp.wait()
    setup(1)
    setup(4)
    for i in COMPS[4:]:
        chunk_dot(0, i)
    for i in COMPS[:2]:
        chunk_dot(1, i)

    for cp in (xr, wc[2], wc[3]):
        cp.wait()
    setup(2)
    for i, k in rems[:6]:
        rem_dot(i, k)

    xe.wait()
    setup(3)
    for i, k in rems[6:]:
        rem_dot(i, k)
    for n in range(P):
        m = [None] * 6
        for idx, i in enumerate(ORDER):
            k0 = 2 if i in COMPS[:2] else 1
            m[i] = (_dot(g_tiles(range(5 * i + k0, 5 * i + NK), fresh=n == 0), t_in(n, i, k0 * L, KF))
                    + acc[i, :, n * L:(n + 1) * L])
            fence(idx)
        finish(n, m, None)

    xh.wait()
    window_wait()
    out_copy(0, 0, 4 * P).start()
    stage(P, ORDER[0])

    def body(it, carry):
        c0 = P + it * NT
        for cp in window(c0 + NT + 1):
            cp.start()
        for u in range(NT - 1):
            finish(c0 + u, matmuls(c0 + u, staged=0 if u == 0 else None), ((0, 4),))
        m = matmuls(c0 + NT - 1, staged=1, restage=True)
        stage(c0 + NT, ORDER[0])
        finish(c0 + NT - 1, m, ((1, 2), (3, 1), (0, 1)))
        window_wait()
        return carry

    lax.fori_loop(0, NIT, body, 0)
    pltpu.make_async_copy(o_hbm, o_hbm, out_sem).wait()


@jax.jit
def pallas_standalone__batchnorm__sampling_kernel(x, w, mean, var, g, b):
    B, S, C = x.shape
    NJ = B // L
    NK = C // L
    assert w.shape == (3, C, C) and C == NK * L + L // 2 and S == 32 and NJ == 8 and NK == 4
    hbm = pl.BlockSpec(memory_space=pl.ANY)
    out = pl.pallas_call(
        _kernel,
        in_specs=[hbm] * 6,
        out_specs=hbm,
        out_shape=jax.ShapeDtypeStruct((S, C, B), x.dtype),
        scratch_shapes=[
            pltpu.VMEM((NJ, S + 2, C, L), bf16),
            pltpu.VMEM((NJ, S, C, L), bf16),
            pltpu.VMEM((3, C, C), bf16),
            *[pltpu.VMEM((C,), bf16)] * 4,
            pltpu.VMEM((6 * (NK + 1), C, L), bf16),
            pltpu.VMEM((6 * (NK + 1), C // 2, L), u32),
            pltpu.VMEM(((NK + 1) * L, L), f32),
            pltpu.VMEM((6, C, P * L), f32),
            pltpu.VMEM((C, L), f32),
            pltpu.VMEM((C, L), f32),
            pltpu.SMEM((1,), jnp.int32),
            pltpu.SemaphoreType.DMA(()),
            pltpu.SemaphoreType.DMA((5,)),
            pltpu.SemaphoreType.DMA((NK + 1,)),
            pltpu.SemaphoreType.DMA(()),
            pltpu.SemaphoreType.DMA(()),
        ],
        compiler_params=pltpu.CompilerParams(
            vmem_limit_bytes=120 * 1024 * 1024,
            disable_bounds_checks=True,
            disable_semaphore_checks=True,
        ),
    )(jnp.transpose(x, (1, 2, 0)), w, mean, var, g, b)
    return jnp.transpose(out, (2, 0, 1))
```

```python
import jax
import jax.numpy as jnp
from jax import lax
import jax.experimental.pallas as pl
import jax.experimental.pallas.tpu as pltpu

f32 = jnp.float32
bf16 = jnp.bfloat16
u32 = jnp.uint32

L = 128
PA = 2.0 / 3.0
PB = 1.5
A2 = PA * PA
B2 = PB * PB
S2 = A2 + B2
NA = 2 * A2 * (A2 - B2)
NB = 2 * B2 * (B2 - A2)

P = 4
NT = 6
ORDER = (1, 2, 3, 4, 5, 0)
COMPS = (0, 5, 1, 2, 3, 4)


def _divmod_pow2(x, n):
    if isinstance(x, int):
        return x // n, x % n
    return lax.shift_right_logical(x, n.bit_length() - 1), lax.bitwise_and(x, n - 1)


def _dot(a, b):
    return jnp.dot(a, b.astype(bf16), preferred_element_type=f32)


def _kernel(x_hbm, w_hbm, mean_hbm, var_hbm, g_hbm, b_hbm, o_hbm,
            xbuf, obuf, wbuf, vb0, vb1, vb2, vb3, gnew, gt, abuf, acc, sc_ref, sh_ref, fence_ref,
            x_sem, p_sems, w_sems, v_sem, out_sem):
    S, C, B = x_hbm.shape
    NJ = B // L
    TPS = S // 4
    NK = C // L
    KF = NK * L
    H = C // 2
    NIT = (NJ * TPS - P) // NT
    PP = 4 * P + 1
    SHARED = 6 * (NK + 1) - 1

    def lanes(j):
        return pl.ds(j * L if isinstance(j, int) else pl.multiple_of(j * L, L), L)

    def x_copy(j, p0, n, sem, r0=0, r1=C):
        return pltpu.make_async_copy(
            x_hbm.at[pl.ds(p0, n), pl.ds(r0, r1 - r0), lanes(j)],
            xbuf.at[j, pl.ds(p0 + 1, n), pl.ds(r0, r1 - r0), :], sem)

    def window(c):
        out = []
        for u, cnt in [(0, 1)] + [(u, 2) for u in range(1, NT - 1, 2)] + [(NT - 1, 1)]:
            j, t = _divmod_pow2(c + u, TPS)
            out.append(x_copy(_divmod_pow2(j, NJ)[1], 4 * t, 4 * cnt, x_sem))
        return out

    def window_wait():
        total = xbuf.at[0, pl.ds(0, 4 * NT)]
        pltpu.make_async_copy(total, total, x_sem).wait()

    def out_copy(n, p0, cnt):
        j, t = _divmod_pow2(n, TPS)
        return pltpu.make_async_copy(
            obuf.at[j, pl.ds(4 * t + p0, cnt)], o_hbm.at[pl.ds(4 * t + p0, cnt), :, lanes(j)], out_sem)

    wc = [pltpu.make_async_copy(w_hbm.at[:, pl.ds(kc * L, min(L, C - kc * L)), :],
                                wbuf.at[:, pl.ds(kc * L, min(L, C - kc * L)), :], w_sems.at[kc])
          for kc in range(NK + 1)]
    vbuf = (vb0, vb1, vb2, vb3)
    vc = [pltpu.make_async_copy(r, vbuf[i], v_sem) for i, r in enumerate((mean_hbm, var_hbm, g_hbm, b_hbm))]
    x0, x1, xe, xr = (x_copy(0, 0, PP, p_sems.at[i], r0, r1)
                      for i, (r0, r1) in enumerate(((0, L), (L, 2 * L), (2 * L, KF), (KF, C))))
    xh = x_copy(0, PP, 3, p_sems.at[4])

    for cp in [wc[0], *vc, x0, wc[1], x1, wc[4], xr, wc[2], wc[3], xe, xh, *window(P + 1)]:
        cp.start()

    for j in range(NJ):
        xbuf[j, 0] = jnp.zeros((C, L), bf16)
        xbuf[j, S + 1] = jnp.zeros((C, L), bf16)

    def setup(kc):
        if kc < NK:
            w0, w1, w2 = (wbuf[k, kc * L:(kc + 1) * L, :].astype(f32).T for k in range(3))
        else:
            r = [wbuf[k, KF:, :].astype(f32) for k in range(3)]
            t0, t1, t2 = (jnp.concatenate(p, axis=0).T for p in ((r[0], -r[0]), (r[1], r[0]), (r[2], r[2])))
            left = lax.broadcasted_iota(jnp.int32, (H, L), 1) < L // 2
            w0 = jnp.concatenate([t0[:H], jnp.where(left, t0[H:], t2[:H])], axis=0)
            w1 = jnp.concatenate([jnp.where(left, t1[:H], t0[H:]), jnp.where(left, t1[H:], t2[H:])], axis=0)
            w2 = jnp.concatenate([jnp.where(left, t2[:H], 0.0), jnp.where(left, t2[H:], 0.0)], axis=0)
            gnew[SHARED, :H, :] = jnp.where(left, t2[:H], t1[H:]).astype(bf16)
        ea = (w0 + A2 * w2) * (1.0 / NA)
        oa = w1 * (PA / NA)
        eb = (w0 + B2 * w2) * (1.0 / NB)
        ob = w1 * (PB / NB)
        for i, gi in enumerate([w0, ea + oa, ea - oa, eb + ob, eb - ob, w2]):
            if kc < NK or 0 < i < 5:
                gnew[5 * i + kc] = gi.astype(bf16)

    def bn_consts():
        mean, var, g, b = (r[...].astype(f32).reshape(1, C) for r in vbuf)
        sc = 0.5 * g * lax.rsqrt(var + 1e-5)
        sh = 0.5 * b - mean * sc
        sc_ref[...] = jnp.broadcast_to(sc, (L, C)).T
        sh_ref[...] = jnp.broadcast_to(sh, (L, C)).T

    def t_in(n, i, lo, hi):
        j, t = _divmod_pow2(n, TPS)
        j = _divmod_pow2(j, NJ)[1]
        d = lambda q: xbuf[j, 4 * t + q, lo:hi, :].astype(f32)
        if i == 0:
            return (d(0) + d(4)) - S2 * d(2)
        if i == 5:
            return (d(1) + d(5)) - S2 * d(3)
        c2, c1, c3 = {1: (B2, -PB, PA), 2: (B2, PB, -PA), 3: (A2, -PA, PB), 4: (A2, PA, -PB)}[i]
        return (d(4) - c2 * d(2)) + (c1 * d(1) + c3 * d(3))

    def rem(n, i, k):
        return jnp.concatenate([t_in(n, i, KF, C), t_in(n, k, KF, C)], axis=0)

    def g_tiles(slots, fresh=False, lo=0, hi=C):
        out = []
        for slot in slots:
            if fresh:
                v = gnew[slot, lo:hi, :]
                gt[slot, lo // 2:hi // 2, :] = pltpu.bitcast(v, u32)
            else:
                v = pltpu.bitcast(gt[slot, lo // 2:hi // 2, :], bf16)
            out.append(v)
        return jnp.concatenate(out, axis=1)

    def fence(v):
        fence_ref[0] = v

    def stage(n, i):
        abuf[:KF, :] = t_in(n, i, 0, KF)
        abuf[KF:, :] = rem(n, i, 0)

    def matmuls(n, staged=None, restage=False):
        m = [None] * 6
        for idx, i in enumerate(ORDER):
            if 0 < i < 5:
                if idx == staged:
                    if restage:
                        stage(n, i)
                    main, top = abuf[:KF, :], abuf[KF:, :]
                else:
                    main, top = t_in(n, i, 0, KF), rem(n, i, 0)
                slots = range(5 * i, 5 * i + NK + 1)
                halves = [_dot(g_tiles(slots, lo=0, hi=H), jnp.concatenate([main, top], axis=0)),
                          _dot(g_tiles(slots, lo=H, hi=C), jnp.concatenate([main, rem(n, i, 5)], axis=0))]
            else:
                mi = _dot(g_tiles(range(5 * i, 5 * i + NK)), t_in(n, i, 0, KF))
                if i == 5:
                    shared = _dot(g_tiles([SHARED], lo=0, hi=H), rem(n, 5, 0))
                halves = [mi[:H] + shared, mi[H:]] if i == 5 else [mi[:H], mi[H:] + shared]
            m[i] = jnp.concatenate(halves, axis=0)
            fence(idx)
        return m

    def finish(n, m, groups):
        j, t = _divmod_pow2(n, TPS)
        sc = sc_ref[...]
        sh = sh_ref[...]
        s12 = m[1] + m[2]
        d12 = m[1] - m[2]
        s34 = m[3] + m[4]
        d34 = m[3] - m[4]
        p = PA * d12
        q = PB * d34
        y = (m[0] + s12 + s34, p + q, A2 * s12 + B2 * s34, A2 * p + B2 * q + m[5])
        for p0, cnt in groups or ((0, 4),):
            for s in range(p0, p0 + cnt):
                h = y[s] * sc + sh
                obuf[j, 4 * t + s] = (h + h * jnp.tanh(h)).astype(bf16)
            if groups:
                out_copy(n, p0, cnt).start()

    def chunk_dot(kc, i):
        r = _dot(g_tiles([5 * i + kc], fresh=True),
                 jnp.concatenate([t_in(n, i, kc * L, (kc + 1) * L) for n in range(P)], axis=1))
        acc[i] = r if kc == 0 else acc[i] + r
        fence(i)

    def rem_dot(i, k):
        lo = 0 if k == 0 else H
        r = _dot(g_tiles([SHARED if i == 5 else 5 * i + NK], fresh=True, lo=lo, hi=lo + H),
                 jnp.concatenate([rem(n, i, k) for n in range(P)], axis=1))
        acc[i, lo:lo + H, :] += r
        if i == 5:
            acc[0, H:, :] += r
        fence(i)

    rems = [(5, 0)] + [(i, k) for i in range(1, 5) for k in (0, 5)]

    for cp in (wc[0], *vc):
        cp.wait()
    setup(0)
    bn_consts()

    x0.wait()
    for i in COMPS[:5]:
        chunk_dot(0, i)

    for cp in (wc[1], x1, wc[4]):
        cp.wait()
    setup(1)
    setup(4)
    chunk_dot(0, COMPS[5])
    for i in COMPS[:2]:
        chunk_dot(1, i)

    for cp in (xr, wc[2], wc[3]):
        cp.wait()
    setup(2)
    for i, k in rems[:7]:
        rem_dot(i, k)

    xe.wait()
    setup(3)
    for i, k in rems[7:]:
        rem_dot(i, k)
    for n in range(P):
        m = [None] * 6
        for idx, i in enumerate(ORDER):
            k0 = 2 if i in COMPS[:2] else 1
            m[i] = (_dot(g_tiles(range(5 * i + k0, 5 * i + NK), fresh=n == 0), t_in(n, i, k0 * L, KF))
                    + acc[i, :, n * L:(n + 1) * L])
            fence(idx)
        finish(n, m, None)

    xh.wait()
    window_wait()
    out_copy(0, 0, 4 * P).start()
    stage(P, ORDER[0])

    def body(it, carry):
        c0 = P + it * NT
        for cp in window(c0 + NT + 1):
            cp.start()
        for u in range(NT - 1):
            finish(c0 + u, matmuls(c0 + u, staged=0 if u == 0 else None), ((0, 4),))
        m = matmuls(c0 + NT - 1, staged=3, restage=True)
        stage(c0 + NT, ORDER[0])
        finish(c0 + NT - 1, m, ((1, 2), (3, 1), (0, 1)))
        window_wait()
        return carry

    lax.fori_loop(0, NIT, body, 0)
    pltpu.make_async_copy(o_hbm, o_hbm, out_sem).wait()


@jax.jit
def pallas_standalone__batchnorm__sampling_kernel(x, w, mean, var, g, b):
    B, S, C = x.shape
    NJ = B // L
    NK = C // L
    assert w.shape == (3, C, C) and C == NK * L + L // 2 and S == 32 and NJ == 8 and NK == 4
    hbm = pl.BlockSpec(memory_space=pl.ANY)
    out = pl.pallas_call(
        _kernel,
        in_specs=[hbm] * 6,
        out_specs=hbm,
        out_shape=jax.ShapeDtypeStruct((S, C, B), x.dtype),
        scratch_shapes=[
            pltpu.VMEM((NJ, S + 2, C, L), bf16),
            pltpu.VMEM((NJ, S, C, L), bf16),
            pltpu.VMEM((3, C, C), bf16),
            *[pltpu.VMEM((C,), bf16)] * 4,
            pltpu.VMEM((6 * (NK + 1), C, L), bf16),
            pltpu.VMEM((6 * (NK + 1), C // 2, L), u32),
            pltpu.VMEM(((NK + 1) * L, L), f32),
            pltpu.VMEM((6, C, P * L), f32),
            pltpu.VMEM((C, L), f32),
            pltpu.VMEM((C, L), f32),
            pltpu.SMEM((1,), jnp.int32),
            pltpu.SemaphoreType.DMA(()),
            pltpu.SemaphoreType.DMA((5,)),
            pltpu.SemaphoreType.DMA((NK + 1,)),
            pltpu.SemaphoreType.DMA(()),
            pltpu.SemaphoreType.DMA(()),
        ],
        compiler_params=pltpu.CompilerParams(
            vmem_limit_bytes=120 * 1024 * 1024,
            disable_bounds_checks=True,
            disable_semaphore_checks=True,
        ),
    )(jnp.transpose(x, (1, 2, 0)), w, mean, var, g, b)
    return jnp.transpose(out, (2, 0, 1))
```

```python
import jax
import jax.numpy as jnp
from jax import lax
import jax.experimental.pallas as pl
import jax.experimental.pallas.tpu as pltpu

f32 = jnp.float32
bf16 = jnp.bfloat16
u32 = jnp.uint32

L = 128
PA = 2.0 / 3.0
PB = 1.5
A2 = PA * PA
B2 = PB * PB
S2 = A2 + B2
NA = 2 * A2 * (A2 - B2)
NB = 2 * B2 * (B2 - A2)

P = 4
NT = 6
ORDER = (1, 2, 3, 4, 5, 0)
COMPS = (0, 5, 1, 2, 3, 4)


def _divmod_pow2(x, n):
    if isinstance(x, int):
        return x // n, x % n
    return lax.shift_right_logical(x, n.bit_length() - 1), lax.bitwise_and(x, n - 1)


def _dot(a, b):
    return jnp.dot(a, b.astype(bf16), preferred_element_type=f32)


def _kernel(x_hbm, w_hbm, mean_hbm, var_hbm, g_hbm, b_hbm, o_hbm,
            xbuf, obuf, wbuf, vb0, vb1, vb2, vb3, gnew, gt, abuf, acc, sc_ref, sh_ref, fence_ref,
            x_sem, p_sems, w_sems, v_sem, out_sem):
    S, C, B = x_hbm.shape
    NJ = B // L
    TPS = S // 4
    NK = C // L
    KF = NK * L
    H = C // 2
    NIT = (NJ * TPS - P) // NT
    PP = 4 * P + 1
    SHARED = 6 * (NK + 1) - 1

    def lanes(j):
        return pl.ds(j * L if isinstance(j, int) else pl.multiple_of(j * L, L), L)

    def x_copy(j, p0, n, sem, r0=0, r1=C):
        return pltpu.make_async_copy(
            x_hbm.at[pl.ds(p0, n), pl.ds(r0, r1 - r0), lanes(j)],
            xbuf.at[j, pl.ds(p0 + 1, n), pl.ds(r0, r1 - r0), :], sem)

    def window(c):
        out = []
        for u, cnt in [(0, 1)] + [(u, 2) for u in range(1, NT - 1, 2)] + [(NT - 1, 1)]:
            j, t = _divmod_pow2(c + u, TPS)
            out.append(x_copy(_divmod_pow2(j, NJ)[1], 4 * t, 4 * cnt, x_sem))
        return out

    def window_wait():
        total = xbuf.at[0, pl.ds(0, 4 * NT)]
        pltpu.make_async_copy(total, total, x_sem).wait()

    def out_copy(n, p0, cnt):
        j, t = _divmod_pow2(n, TPS)
        return pltpu.make_async_copy(
            obuf.at[j, pl.ds(4 * t + p0, cnt)], o_hbm.at[pl.ds(4 * t + p0, cnt), :, lanes(j)], out_sem)

    wc = [pltpu.make_async_copy(w_hbm.at[:, pl.ds(kc * L, min(L, C - kc * L)), :],
                                wbuf.at[:, pl.ds(kc * L, min(L, C - kc * L)), :], w_sems.at[kc])
          for kc in range(NK + 1)]
    vbuf = (vb0, vb1, vb2, vb3)
    vc = [pltpu.make_async_copy(r, vbuf[i], v_sem) for i, r in enumerate((mean_hbm, var_hbm, g_hbm, b_hbm))]
    x0, x1, xe, xr = (x_copy(0, 0, PP, p_sems.at[i], r0, r1)
                      for i, (r0, r1) in enumerate(((0, L), (L, 2 * L), (2 * L, KF), (KF, C))))
    xh = x_copy(0, PP, 3, p_sems.at[4])

    for cp in [wc[4], xr, wc[0], *vc, x0, wc[1], x1, wc[2], wc[3], xe, xh, *window(P + 1)]:
        cp.start()

    for j in range(NJ):
        xbuf[j, 0] = jnp.zeros((C, L), bf16)
        xbuf[j, S + 1] = jnp.zeros((C, L), bf16)

    def setup(kc):
        if kc < NK:
            w0, w1, w2 = (wbuf[k, kc * L:(kc + 1) * L, :].astype(f32).T for k in range(3))
        else:
            r = [wbuf[k, KF:, :].astype(f32) for k in range(3)]
            t0, t1, t2 = (jnp.concatenate(p, axis=0).T for p in ((r[0], -r[0]), (r[1], r[0]), (r[2], r[2])))
            left = lax.broadcasted_iota(jnp.int32, (H, L), 1) < L // 2
            w0 = jnp.concatenate([t0[:H], jnp.where(left, t0[H:], t2[:H])], axis=0)
            w1 = jnp.concatenate([jnp.where(left, t1[:H], t0[H:]), jnp.where(left, t1[H:], t2[H:])], axis=0)
            w2 = jnp.concatenate([jnp.where(left, t2[:H], 0.0), jnp.where(left, t2[H:], 0.0)], axis=0)
            gnew[SHARED, :H, :] = jnp.where(left, t2[:H], t1[H:]).astype(bf16)
        ea = (w0 + A2 * w2) * (1.0 / NA)
        oa = w1 * (PA / NA)
        eb = (w0 + B2 * w2) * (1.0 / NB)
        ob = w1 * (PB / NB)
        for i, gi in enumerate([w0, ea + oa, ea - oa, eb + ob, eb - ob, w2]):
            if kc < NK or 0 < i < 5:
                gnew[5 * i + kc] = gi.astype(bf16)

    def bn_consts():
        mean, var, g, b = (r[...].astype(f32).reshape(1, C) for r in vbuf)
        sc = 0.5 * g * lax.rsqrt(var + 1e-5)
        sh = 0.5 * b - mean * sc
        sc_ref[...] = jnp.broadcast_to(sc, (L, C)).T
        sh_ref[...] = jnp.broadcast_to(sh, (L, C)).T

    def t_in(n, i, lo, hi):
        j, t = _divmod_pow2(n, TPS)
        j = _divmod_pow2(j, NJ)[1]
        d = lambda q: xbuf[j, 4 * t + q, lo:hi, :].astype(f32)
        if i == 0:
            return (d(0) + d(4)) - S2 * d(2)
        if i == 5:
            return (d(1) + d(5)) - S2 * d(3)
        c2, c1, c3 = {1: (B2, -PB, PA), 2: (B2, PB, -PA), 3: (A2, -PA, PB), 4: (A2, PA, -PB)}[i]
        return (d(4) - c2 * d(2)) + (c1 * d(1) + c3 * d(3))

    def rem(n, i, k):
        return jnp.concatenate([t_in(n, i, KF, C), t_in(n, k, KF, C)], axis=0)

    def g_tiles(slots, fresh=False, lo=0, hi=C):
        out = []
        for slot in slots:
            if fresh:
                v = gnew[slot, lo:hi, :]
                gt[slot, lo // 2:hi // 2, :] = pltpu.bitcast(v, u32)
            else:
                v = pltpu.bitcast(gt[slot, lo // 2:hi // 2, :], bf16)
            out.append(v)
        return jnp.concatenate(out, axis=1)

    def fence(v):
        fence_ref[0] = v

    def stage(n, i):
        abuf[:KF, :] = t_in(n, i, 0, KF)
        abuf[KF:, :] = rem(n, i, 0)

    def matmuls(n, staged=None, restage=False):
        m = [None] * 6
        for idx, i in enumerate(ORDER):
            if 0 < i < 5:
                if idx == staged:
                    if restage:
                        stage(n, i)
                    main, top = abuf[:KF, :], abuf[KF:, :]
                else:
                    main, top = t_in(n, i, 0, KF), rem(n, i, 0)
                slots = range(5 * i, 5 * i + NK + 1)
                halves = [_dot(g_tiles(slots, lo=0, hi=H), jnp.concatenate([main, top], axis=0)),
                          _dot(g_tiles(slots, lo=H, hi=C), jnp.concatenate([main, rem(n, i, 5)], axis=0))]
            else:
                mi = _dot(g_tiles(range(5 * i, 5 * i + NK)), t_in(n, i, 0, KF))
                if i == 5:
                    shared = _dot(g_tiles([SHARED], lo=0, hi=H), rem(n, 5, 0))
                halves = [mi[:H] + shared, mi[H:]] if i == 5 else [mi[:H], mi[H:] + shared]
            m[i] = jnp.concatenate(halves, axis=0)
            fence(idx)
        return m

    def finish(n, m, groups):
        j, t = _divmod_pow2(n, TPS)
        sc = sc_ref[...]
        sh = sh_ref[...]
        s12 = m[1] + m[2]
        d12 = m[1] - m[2]
        s34 = m[3] + m[4]
        d34 = m[3] - m[4]
        p = PA * d12
        q = PB * d34
        y = (m[0] + s12 + s34, p + q, A2 * s12 + B2 * s34, A2 * p + B2 * q + m[5])
        for p0, cnt in groups or ((0, 4),):
            for s in range(p0, p0 + cnt):
                h = y[s] * sc + sh
                obuf[j, 4 * t + s] = (h + h * jnp.tanh(h)).astype(bf16)
            if groups:
                out_copy(n, p0, cnt).start()

    started = set()

    def accumulate(i, lo, r):
        if (i, lo) in started:
            acc[i, lo:lo + H, :] += r
        else:
            acc[i, lo:lo + H, :] = r
            started.add((i, lo))

    def chunk_dot(kc, i):
        r = _dot(g_tiles([5 * i + kc], fresh=True),
                 jnp.concatenate([t_in(n, i, kc * L, (kc + 1) * L) for n in range(P)], axis=1))
        accumulate(i, 0, r[:H])
        accumulate(i, H, r[H:])
        fence(i)

    def rem_dot(i, k):
        lo = 0 if k == 0 else H
        r = _dot(g_tiles([SHARED if i == 5 else 5 * i + NK], fresh=True, lo=lo, hi=lo + H),
                 jnp.concatenate([rem(n, i, k) for n in range(P)], axis=1))
        accumulate(i, lo, r)
        if i == 5:
            accumulate(0, H, r)
        fence(i)

    rems = [(5, 0)] + [(i, k) for i in range(1, 5) for k in (0, 5)]

    wc[4].wait()
    setup(4)

    xr.wait()
    for i, k in rems[:3]:
        rem_dot(i, k)

    wc[0].wait()
    setup(0)
    for i, k in rems[3:]:
        rem_dot(i, k)

    for cp in (x0, wc[1], *vc):
        cp.wait()
    setup(1)
    bn_consts()
    for i in COMPS:
        chunk_dot(0, i)

    for cp in (x1, wc[2], wc[3]):
        cp.wait()
    setup(2)
    setup(3)
    for i in COMPS[:2]:
        chunk_dot(1, i)

    xe.wait()
    for n in range(P):
        m = [None] * 6
        for idx, i in enumerate(ORDER):
            k0 = 2 if i in COMPS[:2] else 1
            m[i] = (_dot(g_tiles(range(5 * i + k0, 5 * i + NK), fresh=n == 0), t_in(n, i, k0 * L, KF))
                    + acc[i, :, n * L:(n + 1) * L])
            fence(idx)
        finish(n, m, None)

    xh.wait()
    window_wait()
    out_copy(0, 0, 4 * P).start()
    stage(P, ORDER[0])

    def body(it, carry):
        c0 = P + it * NT
        for cp in window(c0 + NT + 1):
            cp.start()
        for u in range(NT - 1):
            finish(c0 + u, matmuls(c0 + u, staged=0 if u == 0 else None), ((0, 4),))
        m = matmuls(c0 + NT - 1, staged=3, restage=True)
        stage(c0 + NT, ORDER[0])
        finish(c0 + NT - 1, m, ((1, 2), (3, 1), (0, 1)))
        window_wait()
        return carry

    lax.fori_loop(0, NIT, body, 0)
    pltpu.make_async_copy(o_hbm, o_hbm, out_sem).wait()


@jax.jit
def pallas_standalone__batchnorm__sampling_kernel(x, w, mean, var, g, b):
    B, S, C = x.shape
    NJ = B // L
    NK = C // L
    assert w.shape == (3, C, C) and C == NK * L + L // 2 and S == 32 and NJ == 8 and NK == 4
    hbm = pl.BlockSpec(memory_space=pl.ANY)
    out = pl.pallas_call(
        _kernel,
        in_specs=[hbm] * 6,
        out_specs=hbm,
        out_shape=jax.ShapeDtypeStruct((S, C, B), x.dtype),
        scratch_shapes=[
            pltpu.VMEM((NJ, S + 2, C, L), bf16),
            pltpu.VMEM((NJ, S, C, L), bf16),
            pltpu.VMEM((3, C, C), bf16),
            *[pltpu.VMEM((C,), bf16)] * 4,
            pltpu.VMEM((6 * (NK + 1), C, L), bf16),
            pltpu.VMEM((6 * (NK + 1), C // 2, L), u32),
            pltpu.VMEM(((NK + 1) * L, L), f32),
            pltpu.VMEM((6, C, P * L), f32),
            pltpu.VMEM((C, L), f32),
            pltpu.VMEM((C, L), f32),
            pltpu.SMEM((1,), jnp.int32),
            pltpu.SemaphoreType.DMA(()),
            pltpu.SemaphoreType.DMA((5,)),
            pltpu.SemaphoreType.DMA((NK + 1,)),
            pltpu.SemaphoreType.DMA(()),
            pltpu.SemaphoreType.DMA(()),
        ],
        compiler_params=pltpu.CompilerParams(
            vmem_limit_bytes=120 * 1024 * 1024,
            disable_bounds_checks=True,
            disable_semaphore_checks=True,
        ),
    )(jnp.transpose(x, (1, 2, 0)), w, mean, var, g, b)
    return jnp.transpose(out, (2, 0, 1))
```

```python
import jax
import jax.numpy as jnp
from jax import lax
import jax.experimental.pallas as pl
import jax.experimental.pallas.tpu as pltpu

f32 = jnp.float32
bf16 = jnp.bfloat16
u32 = jnp.uint32

L = 128
PA = 2.0 / 3.0
PB = 1.5
A2 = PA * PA
B2 = PB * PB
S2 = A2 + B2
NA = 2 * A2 * (A2 - B2)
NB = 2 * B2 * (B2 - A2)

RS = 384
P = 4
NT = 6
ORDER = (1, 2, 3, 4, 5, 0)
COMPS = (0, 5, 1, 2, 3, 4)


def _divmod_pow2(x, n):
    if isinstance(x, int):
        return x // n, x % n
    return lax.shift_right_logical(x, n.bit_length() - 1), lax.bitwise_and(x, n - 1)


def _dot(a, b):
    return jnp.dot(a, b.astype(bf16), preferred_element_type=f32)


def _kernel(x_hbm, w_hbm, mean_hbm, var_hbm, g_hbm, b_hbm, o_hbm,
            xbuf, obuf, wbuf, vb0, vb1, vb2, vb3, gnew, gt, abuf, acc, sc_ref, sh_ref, fence_ref,
            x_sem, p_sems, w_sems, v_sem, out_sem):
    S, C, B = x_hbm.shape
    NJ = B // L
    TPS = S // 4
    NK = C // L
    KF = NK * L
    H = C // 2
    NIT = (NJ * TPS - P) // NT
    PP = 4 * P + 1
    SHARED = 6 * (NK + 1) - 1

    def lanes(j):
        return pl.ds(j * L if isinstance(j, int) else pl.multiple_of(j * L, L), L)

    def x_copy(j, p0, n, sem, r0=0, r1=C):
        return pltpu.make_async_copy(
            x_hbm.at[pl.ds(p0, n), pl.ds(r0, r1 - r0), lanes(j)],
            xbuf.at[j, pl.ds(p0 + 1, n), pl.ds(r0, r1 - r0), :], sem)

    def window(c):
        out = []
        for u, cnt in [(0, 1)] + [(u, 2) for u in range(1, NT - 1, 2)] + [(NT - 1, 1)]:
            j, t = _divmod_pow2(c + u, TPS)
            out.append(x_copy(_divmod_pow2(j, NJ)[1], 4 * t, 4 * cnt, x_sem))
        return out

    def window_wait():
        total = xbuf.at[0, pl.ds(0, 4 * NT)]
        pltpu.make_async_copy(total, total, x_sem).wait()

    def out_copy(n, p0, cnt, r0=0, r1=C):
        j, t = _divmod_pow2(n, TPS)
        return pltpu.make_async_copy(
            obuf.at[j, pl.ds(4 * t + p0, cnt), pl.ds(r0, r1 - r0), :],
            o_hbm.at[pl.ds(4 * t + p0, cnt), pl.ds(r0, r1 - r0), lanes(j)], out_sem)

    wc = [pltpu.make_async_copy(w_hbm.at[:, pl.ds(kc * L, min(L, C - kc * L)), :],
                                wbuf.at[:, pl.ds(kc * L, min(L, C - kc * L)), :], w_sems.at[kc])
          for kc in range(NK + 1)]
    vbuf = (vb0, vb1, vb2, vb3)
    vc = [pltpu.make_async_copy(r, vbuf[i], v_sem) for i, r in enumerate((mean_hbm, var_hbm, g_hbm, b_hbm))]
    x0, x1, xe, xr = (x_copy(0, 0, PP, p_sems.at[i], r0, r1)
                      for i, (r0, r1) in enumerate(((0, L), (L, 2 * L), (2 * L, KF), (KF, C))))
    xh = x_copy(0, PP, 3, p_sems.at[4])

    for cp in [wc[4], xr, wc[0], *vc, x0, wc[1], x1, wc[2], wc[3], xe, xh, *window(P + 1)]:
        cp.start()

    for j in range(NJ):
        xbuf[j, 0] = jnp.zeros((C, L), bf16)
        xbuf[j, S + 1] = jnp.zeros((C, L), bf16)

    def setup(kc):
        if kc < NK:
            w0, w1, w2 = (wbuf[k, kc * L:(kc + 1) * L, :].astype(f32).T for k in range(3))
        else:
            r = [wbuf[k, KF:, :].astype(f32) for k in range(3)]
            t0, t1, t2 = (jnp.concatenate(p, axis=0).T for p in ((r[0], -r[0]), (r[1], r[0]), (r[2], r[2])))
            left = lax.broadcasted_iota(jnp.int32, (H, L), 1) < L // 2
            w0 = jnp.concatenate([t0[:H], jnp.where(left, t0[H:], t2[:H])], axis=0)
            w1 = jnp.concatenate([jnp.where(left, t1[:H], t0[H:]), jnp.where(left, t1[H:], t2[H:])], axis=0)
            w2 = jnp.concatenate([jnp.where(left, t2[:H], 0.0), jnp.where(left, t2[H:], 0.0)], axis=0)
            gnew[SHARED, :H, :] = jnp.where(left, t2[:H], t1[H:]).astype(bf16)
        ea = (w0 + A2 * w2) * (1.0 / NA)
        oa = w1 * (PA / NA)
        eb = (w0 + B2 * w2) * (1.0 / NB)
        ob = w1 * (PB / NB)
        for i, gi in enumerate([w0, ea + oa, ea - oa, eb + ob, eb - ob, w2]):
            if kc < NK or 0 < i < 5:
                gnew[5 * i + kc] = gi.astype(bf16)

    def bn_consts():
        mean, var, g, b = (r[...].astype(f32).reshape(1, C) for r in vbuf)
        sc = 0.5 * g * lax.rsqrt(var + 1e-5)
        sh = 0.5 * b - mean * sc
        sc_ref[...] = jnp.broadcast_to(sc, (L, C)).T
        sh_ref[...] = jnp.broadcast_to(sh, (L, C)).T

    def t_in(n, i, lo, hi):
        j, t = _divmod_pow2(n, TPS)
        j = _divmod_pow2(j, NJ)[1]
        d = lambda q: xbuf[j, 4 * t + q, lo:hi, :].astype(f32)
        if i == 0:
            return (d(0) + d(4)) - S2 * d(2)
        if i == 5:
            return (d(1) + d(5)) - S2 * d(3)
        c2, c1, c3 = {1: (B2, -PB, PA), 2: (B2, PB, -PA), 3: (A2, -PA, PB), 4: (A2, PA, -PB)}[i]
        return (d(4) - c2 * d(2)) + (c1 * d(1) + c3 * d(3))

    def rem(n, i, k):
        return jnp.concatenate([t_in(n, i, KF, C), t_in(n, k, KF, C)], axis=0)

    def g_tiles(slots, fresh=False, lo=0, hi=C):
        out = []
        for slot in slots:
            if fresh:
                v = gnew[slot, lo:hi, :]
                gt[slot, lo // 2:hi // 2, :] = pltpu.bitcast(v, u32)
            else:
                v = pltpu.bitcast(gt[slot, lo // 2:hi // 2, :], bf16)
            out.append(v)
        return jnp.concatenate(out, axis=1)

    def fence(v):
        fence_ref[0] = v

    def stage(n, i):
        abuf[:KF, :] = t_in(n, i, 0, KF)
        abuf[KF:, :] = rem(n, i, 0)

    def matmuls(n, staged=None, restage=False):
        m = [None] * 6
        for idx, i in enumerate(ORDER):
            if 0 < i < 5:
                if idx == staged:
                    if restage:
                        stage(n, i)
                    main, top = abuf[:KF, :], abuf[KF:, :]
                else:
                    main, top = t_in(n, i, 0, KF), rem(n, i, 0)
                slots = range(5 * i, 5 * i + NK + 1)
                halves = [_dot(g_tiles(slots, lo=0, hi=H), jnp.concatenate([main, top], axis=0)),
                          _dot(g_tiles(slots, lo=H, hi=C), jnp.concatenate([main, rem(n, i, 5)], axis=0))]
            else:
                mi = _dot(g_tiles(range(5 * i, 5 * i + NK)), t_in(n, i, 0, KF))
                if i == 5:
                    shared = _dot(g_tiles([SHARED], lo=0, hi=H), rem(n, 5, 0))
                halves = [mi[:H] + shared, mi[H:]] if i == 5 else [mi[:H], mi[H:] + shared]
            m[i] = jnp.concatenate(halves, axis=0)
            fence(idx)
        return m

    def finish(n, m, groups):
        j, t = _divmod_pow2(n, TPS)
        sc = sc_ref[...]
        sh = sh_ref[...]
        s12 = m[1] + m[2]
        d12 = m[1] - m[2]
        s34 = m[3] + m[4]
        d34 = m[3] - m[4]
        p = PA * d12
        q = PB * d34
        y = (m[0] + s12 + s34, p + q, A2 * s12 + B2 * s34, A2 * p + B2 * q + m[5])
        for p0, cnt, r0, r1 in groups or ((0, 4, 0, C),):
            for s in range(p0, p0 + cnt):
                h = y[s][r0:r1] * sc[r0:r1] + sh[r0:r1]
                obuf[j, 4 * t + s, r0:r1, :] = (h + h * jnp.tanh(h)).astype(bf16)
            if groups:
                out_copy(n, p0, cnt, r0, r1).start()

    started = set()

    def accumulate(i, lo, r):
        if (i, lo) in started:
            acc[i, lo:lo + H, :] += r
        else:
            acc[i, lo:lo + H, :] = r
            started.add((i, lo))

    def chunk_dot(kc, i):
        r = _dot(g_tiles([5 * i + kc], fresh=True),
                 jnp.concatenate([t_in(n, i, kc * L, (kc + 1) * L) for n in range(P)], axis=1))
        accumulate(i, 0, r[:H])
        accumulate(i, H, r[H:])
        fence(i)

    def rem_dot(i, k):
        lo = 0 if k == 0 else H
        r = _dot(g_tiles([SHARED if i == 5 else 5 * i + NK], fresh=True, lo=lo, hi=lo + H),
                 jnp.concatenate([rem(n, i, k) for n in range(P)], axis=1))
        accumulate(i, lo, r)
        if i == 5:
            accumulate(0, H, r)
        fence(i)

    rems = [(5, 0)] + [(i, k) for i in range(1, 5) for k in (0, 5)]

    wc[4].wait()
    setup(4)

    xr.wait()
    for i, k in rems[:6]:
        rem_dot(i, k)

    for cp in (wc[0], x0, *vc):
        cp.wait()
    setup(0)
    bn_consts()
    for i, k in rems[6:8]:
        rem_dot(i, k)
    for i in COMPS[:4]:
        chunk_dot(0, i)

    for cp in (wc[1], x1, wc[2]):
        cp.wait()
    setup(1)
    setup(2)
    for i in COMPS[4:]:
        chunk_dot(0, i)
    for i in COMPS[:2]:
        chunk_dot(1, i)

    for cp in (xe, wc[3]):
        cp.wait()
    setup(3)
    rem_dot(*rems[8])
    for n in range(P):
        m = [None] * 6
        for idx, i in enumerate(ORDER):
            k0 = 2 if i in COMPS[:2] else 1
            m[i] = (_dot(g_tiles(range(5 * i + k0, 5 * i + NK), fresh=n == 0), t_in(n, i, k0 * L, KF))
                    + acc[i, :, n * L:(n + 1) * L])
            fence(idx)
        finish(n, m, None)

    xh.wait()
    window_wait()
    out_copy(0, 0, 4 * P).start()
    stage(P, ORDER[0])

    def body(it, carry):
        c0 = P + it * NT
        for cp in window(c0 + NT + 1):
            cp.start()
        for u in range(NT - 1):
            finish(c0 + u, matmuls(c0 + u, staged=0 if u == 0 else None), ((0, 4, 0, C),))
        m = matmuls(c0 + NT - 1, staged=3, restage=True)
        stage(c0 + NT, ORDER[0])
        finish(c0 + NT - 1, m, ((1, 2, 0, C), (3, 1, 0, C), (0, 1, 0, RS), (0, 1, RS, C)))
        window_wait()
        return carry

    lax.fori_loop(0, NIT, body, 0)
    pltpu.make_async_copy(o_hbm, o_hbm, out_sem).wait()


@jax.jit
def pallas_standalone__batchnorm__sampling_kernel(x, w, mean, var, g, b):
    B, S, C = x.shape
    NJ = B // L
    NK = C // L
    assert w.shape == (3, C, C) and C == NK * L + L // 2 and S == 32 and NJ == 8 and NK == 4
    hbm = pl.BlockSpec(memory_space=pl.ANY)
    out = pl.pallas_call(
        _kernel,
        in_specs=[hbm] * 6,
        out_specs=hbm,
        out_shape=jax.ShapeDtypeStruct((S, C, B), x.dtype),
        scratch_shapes=[
            pltpu.VMEM((NJ, S + 2, C, L), bf16),
            pltpu.VMEM((NJ, S, C, L), bf16),
            pltpu.VMEM((3, C, C), bf16),
            *[pltpu.VMEM((C,), bf16)] * 4,
            pltpu.VMEM((6 * (NK + 1), C, L), bf16),
            pltpu.VMEM((6 * (NK + 1), C // 2, L), u32),
            pltpu.VMEM(((NK + 1) * L, L), f32),
            pltpu.VMEM((6, C, P * L), f32),
            pltpu.VMEM((C, L), f32),
            pltpu.VMEM((C, L), f32),
            pltpu.SMEM((1,), jnp.int32),
            pltpu.SemaphoreType.DMA(()),
            pltpu.SemaphoreType.DMA((5,)),
            pltpu.SemaphoreType.DMA((NK + 1,)),
            pltpu.SemaphoreType.DMA(()),
            pltpu.SemaphoreType.DMA(()),
        ],
        compiler_params=pltpu.CompilerParams(
            vmem_limit_bytes=120 * 1024 * 1024,
            disable_bounds_checks=True,
            disable_semaphore_checks=True,
        ),
    )(jnp.transpose(x, (1, 2, 0)), w, mean, var, g, b)
    return jnp.transpose(out, (2, 0, 1))
```
